```python
import jax
import jax.numpy as jnp

def _softmax(x, axis=-1):
    return jax.nn.softmax(x, axis=axis)

def _gelu(x):
    return jax.nn.gelu(x, approximate=True)

def _silu(x):
    return jax.nn.silu(x)

def _sigmoid(x):
    return jax.nn.sigmoid(x)

def _layernorm(x, axis=-1, eps=1e-05):
    m = jnp.mean(x, axis=axis, keepdims=True)
    v = jnp.var(x, axis=axis, keepdims=True)
    return (x - m) / jnp.sqrt(v + eps)

def _scatter_add(tgt, idx, src, axis=0):
    return tgt.at[idx].add(src)

def _segment_sum(src, seg, n):
    return jax.ops.segment_sum(src, seg, n)

class _Rng:

    def __init__(self, key):
        self._k = key

    def _next(self):
        self._k, sub = jax.random.split(self._k)
        return sub

    def normal(self, shape):
        return jax.random.normal(self._next(), shape, dtype=jnp.bfloat16)

    def randint(self, lo, hi, shape):
        return jax.random.randint(self._next(), shape, lo, hi, dtype=jnp.int32)

    def uniform(self, shape, lo=0.0, hi=1.0):
        return jax.random.uniform(self._next(), shape, jnp.bfloat16, lo, hi)

    def permutation(self, n):
        return jax.random.permutation(self._next(), n)
kernel_name = 'standalone__conformer_family_branchformer__speech'

def setup_inputs():
    _rng = _Rng(jax.random.key(int.from_bytes(__import__("os").urandom(4), "little")))
    _w = lambda a: (lambda t: t.astype(jnp.bfloat16) if jnp.issubdtype(t.dtype, jnp.floating) else t)(jnp.asarray(a))
    B, T, D, K = (2, 4000, 512, 31)
    s = float(D) ** (-0.5)
    return {'x': _w((lambda *s: _rng.normal(s) * 0.05)(B, T, D)), 'w_q': _w((lambda *s: _rng.normal(s) * 0.05)(D, D) * s), 'w_k': _w((lambda *s: _rng.normal(s) * 0.05)(D, D) * s), 'w_v': _w((lambda *s: _rng.normal(s) * 0.05)(D, D) * s), 'w_ao': _w((lambda *s: _rng.normal(s) * 0.05)(D, D) * s), 'w_up': _w((lambda *s: _rng.normal(s) * 0.05)(D, 2 * D) * s), 'dw': _w((lambda *s: _rng.normal(s) * 0.05)(K, D) * (1.0 / K)), 'w_dn': _w((lambda *s: _rng.normal(s) * 0.05)(D, D) * s), 'w_merge': _w((lambda *s: _rng.normal(s) * 0.05)(2 * D, D) * s)}

def reference(x, w_q, w_k, w_v, w_ao, w_up, dw, w_dn, w_merge):
    B, T, D = x.shape
    K = dw.shape[0]
    xa = _layernorm(x, axis=-1)
    q = jnp.einsum('btd,de->bte', xa, w_q)
    k = jnp.einsum('btd,de->bte', xa, w_k)
    v = jnp.einsum('btd,de->bte', xa, w_v)
    logits = jnp.einsum('btd,bsd->bts', q, k) * float(D) ** (-0.5)
    attn = _softmax(logits, axis=-1)
    ya = jnp.einsum('bts,bsd->btd', attn, v)
    ya = jnp.einsum('btd,de->bte', ya, w_ao)
    xc = _layernorm(x, axis=-1)
    h = _gelu(jnp.einsum('btd,de->bte', xc, w_up))
    u = h[..., :D].copy()
    g = _layernorm(h[..., D:], axis=-1)
    pad = K // 2
    gp = jnp.pad(g, ((0, 0), (pad, pad), (0, 0)))
    conv = jnp.zeros_like(g)
    for i in range(K):
        conv = conv + gp[:, i:i + T, :] * dw[i][None, None, :]
    yc = jnp.einsum('btd,de->bte', u * conv, w_dn)
    merged = jnp.concatenate([ya, yc], axis=-1)
    out = jnp.einsum('btf,fd->btd', merged, w_merge)
    return x + out
```

```python
import functools
import math

import jax
import jax.numpy as jnp
import jax.experimental.pallas as pl
import jax.experimental.pallas.tpu as pltpu

_EPS = 1e-5
_LANES = 128
_BLK = 400
_CHUNK = 512
_HALO = 16
_GELU_C = math.sqrt(2.0 / math.pi)
_PIN = True
_CONV_AT = 4
_UNROLL = 4

_F32 = jnp.float32
_BF16 = jnp.bfloat16


def _dot(a, b):
    return jax.lax.dot_general(a, b, (((1,), (0,)), ((), ())), preferred_element_type=_F32)


def _dot_nt(a, b):
    return jax.lax.dot_general(a, b, (((1,), (1,)), ((), ())), preferred_element_type=_F32)


def _layernorm(x):
    m = jnp.mean(x, axis=-1, keepdims=True)
    xc = x - m
    v = jnp.mean(xc * xc, axis=-1, keepdims=True)
    return xc * jax.lax.rsqrt(v + _EPS)


def _gelu(x):
    inner = x * (_GELU_C + (_GELU_C * 0.044715) * (x * x))
    hx = 0.5 * x
    return hx + hx * jnp.tanh(inner)


def _fold_lanes(x, op):
    out = x[:, :_LANES]
    for t in range(1, x.shape[1] // _LANES):
        out = op(out, x[:, t * _LANES:(t + 1) * _LANES])
    return out


def _kernel(x_hbm, wq_hbm, wk_hbm, wv_hbm, wao_hbm, wup_hbm, dw_hbm, wdn_hbm, wm_hbm,
            o_ref,
            x_v, wq_v, wk_v, wup_v, dw_v, w_v,
            a_v, dwf_v, xa_v, g_v, u_v, s_v, m_v, l_v, acc_v, uc_v, q_v, idx_s, sems,
            *, B, T, D, K):
    M, C = _BLK, _CHUNK
    nblk = T // M
    total = B * nblk
    TP = pl.cdiv(T, C) * C
    nchunk = TP // C
    TG = T + 2 * _HALO
    nl = D // _LANES
    step = pl.program_id(0)

    def blk_pos(n):
        if isinstance(n, int):
            return n // nblk, (n % nblk) * M
        b = n // nblk
        return b, pl.multiple_of((n - b * nblk) * M, 16)

    def al(v, mult):
        return v if isinstance(v, int) else pl.multiple_of(v, mult)

    def norm_rows(b, r0, rows):
        xs = x_v[pl.ds(al(b * T + r0, 16), rows), :].astype(_F32)
        xa_v[pl.ds(al(b * TP + r0, 16), rows), :] = _layernorm(xs).astype(_BF16)

    def stage_q(n):
        b, r0 = blk_pos(n)
        xq = xa_v[pl.ds(al(b * TP + r0, 16), M), :]
        return xq, _dot(xq, a_v[...]).astype(_BF16)

    def stage_up(n, xq):
        b, r0 = blk_pos(n)
        u = _gelu(_dot(xq, wup_v[:, :D]))
        for t in range(nl):
            u_v[n % 2, t] = u[:, t * _LANES:(t + 1) * _LANES]
        g = _layernorm(_gelu(_dot(xq, wup_v[:, D:])))
        for t in range(nl):
            g_v[t, pl.ds(al(b * TG + _HALO + r0, 8), M), :] = g[:, t * _LANES:(t + 1) * _LANES]

    def logits_chunk(n, q, j, slot, mx, mask):
        b, _ = blk_pos(n)
        s = _dot_nt(q, xa_v[pl.ds(al(b * TP + j * C, C), C), :])
        if mask:
            col = jax.lax.broadcasted_iota(jnp.int32, s.shape, 1)
            s = jnp.where(col < T - j * C, s, -jnp.inf)
        s_v[slot] = s
        cm = _fold_lanes(s, jnp.maximum)
        return cm if mx is None else jnp.maximum(mx, cm)

    def finish_max(mx):
        m_v[...] = jnp.broadcast_to(jnp.max(mx, axis=-1, keepdims=True), mx.shape)

    def exp_chunk(slot, m, l):
        p = jnp.exp2(s_v[slot] - jnp.tile(m, (1, C // _LANES)))
        cl = _fold_lanes(p, jnp.add)
        return p.astype(_BF16), (cl if l is None else l + cl)

    def pv_chunk(c, j, p, acc):
        b, _ = blk_pos(c)
        pv = _dot(p, xa_v[pl.ds(al(b * TP + j * C, C), C), :])
        return pv if acc is None else acc + pv

    def conv_tile(c, t):
        b, r0 = blk_pos(c)
        base = al(b * TG + r0, 8)
        off = _HALO - K // 2
        conv = None
        for i in range(K):
            term = g_v[t, pl.ds(base + off + i, M), :] * dwf_v[t, i:i + 1, :]
            conv = term if conv is None else conv + term
        return (u_v[c % 2, t] * conv).astype(_BF16)

    def stage_out(c, acc, l, uc):
        b, r0 = blk_pos(c)
        ya = (acc * (1.0 / jnp.sum(l, axis=-1, keepdims=True))).astype(_BF16)
        out = _dot(uc, w_v[7]) + _dot(ya, w_v[6])
        xr = x_v[pl.ds(al(b * T + r0, 16), M), :].astype(_F32)
        o_ref[0] = (xr + out).astype(o_ref.dtype)

    @pl.when(step == 0)
    def _():
        def cp(src, dst, i):
            return pltpu.make_async_copy(src, dst, sems.at[i])

        def cx(j):
            r = al(j * C, C)
            return cp(x_hbm.at[pl.ds(r, C), :], x_v.at[pl.ds(r, C), :], 10 + j)

        c_wq, c_wk, c_wup = cp(wq_hbm, wq_v, 0), cp(wk_hbm, wk_v, 1), cp(wup_hbm, wup_v, 2)
        c_w = [cp(wv_hbm, w_v.at[0], 3), cp(wao_hbm, w_v.at[3], 4), cp(wdn_hbm, w_v.at[1], 5),
               cp(wm_hbm.at[pl.ds(D, D), :], w_v.at[4], 6), cp(wm_hbm.at[pl.ds(0, D), :], w_v.at[5], 7)]
        c_dw = cp(dw_hbm, dw_v, 8)
        c_rest = cp(x_hbm.at[pl.ds(TP, B * T - TP), :], x_v.at[pl.ds(TP, B * T - TP), :], 9)
        for c in [c_wq, c_wk, cx(0), c_wup] + [cx(j) for j in range(1, nchunk)] + c_w + [c_dw, c_rest]:
            c.start()

        for j in range(nchunk):
            idx_s[j] = j
        for b in range(B):
            for t in range(nl):
                g_v[t, b * TG:b * TG + _HALO, :] = jnp.zeros((_HALO, _LANES), _F32)
                g_v[t, (b + 1) * TG - _HALO:(b + 1) * TG, :] = jnp.zeros((_HALO, _LANES), _F32)
        m_v[...] = jnp.full(m_v.shape, -jnp.inf, _F32)

        c_wq.wait()
        c_wk.wait()
        scale = float(D) ** -0.5 * math.log2(math.e)
        a_v[...] = (_dot_nt(wq_v[...], wk_v[...]) * scale).astype(_BF16)
        cx(0).wait()
        norm_rows(0, 0, C)
        xq, q = stage_q(0)
        q_v[...] = q
        c_wup.wait()
        stage_up(0, xq)

        def qk_body(it, carry):
            mx = m_v[...]
            for jj in range(_UNROLL):
                j = it * _UNROLL + jj
                if jj + 1 < _UNROLL:
                    cx(j + 1).wait()
                else:
                    pl.when(j + 1 < nchunk)(lambda: cx(j + 1).wait())
            for jj in range(_UNROLL):
                j = it * _UNROLL + jj
                mx = logits_chunk(0, q_v[...], j, j, mx, jj == _UNROLL - 1)
                norm_rows(0, pl.multiple_of(jnp.minimum(j + 1, nchunk - 1) * C, C), C)
            m_v[...] = mx
            return carry

        jax.lax.fori_loop(0, nchunk // _UNROLL, qk_body, 0)
        finish_max(m_v[...])
        for b in range(B):
            xa_v[b * TP + T:(b + 1) * TP, :] = jnp.zeros((TP - T, D), _BF16)
        for c in c_w:
            c.wait()

        def fold_body(i, carry):
            w_v[jnp.where(i == 0, 2, 8 - i)] = _dot(w_v[i], w_v[3 + i]).astype(_BF16)
            return carry

        jax.lax.fori_loop(0, 3, fold_body, 0)
        c_dw.wait()
        for t in range(nl):
            dwf_v[t] = dw_v[:, t * _LANES:(t + 1) * _LANES].astype(_F32)
        c_rest.wait()
        for b in range(1, B):
            norm_rows(b, 0, M)

    @pl.when(jnp.logical_and(step > 0, step < total))
    def _():
        n, c = step, step - 1
        slot = [idx_s[j] if _PIN else j for j in range(nchunk)]
        slot2 = [idx_s[j] if _PIN else j for j in range(nchunk)]
        xq, q = stage_q(n)
        m = m_v[...]
        p, l = exp_chunk(slot[0], m, None)
        acc = pv_chunk(c, 0, p, None)
        stage_up(n, xq)
        mx = None
        for j in range(nchunk):
            if j + 1 < nchunk:
                p, l = exp_chunk(slot[j + 1], m, l)
            mx = logits_chunk(n, q, j, slot2[j], mx, j == nchunk - 1)
            if j + 1 < nchunk:
                acc = pv_chunk(c, j + 1, p, acc)
            if j == _CONV_AT:
                uc = jnp.concatenate([conv_tile(c, t) for t in range(nl)], axis=1)
        finish_max(mx)
        stage_out(c, acc, l, uc)
        for b in range(1, B):
            norm_rows(b, pl.multiple_of(jnp.minimum(step, nblk - 1) * M, 16), M)

    @pl.when(step == total)
    def _():
        c = total - 1
        nit = nchunk // _UNROLL
        l_v[...] = jnp.zeros(l_v.shape, _F32)
        acc_v[...] = jnp.zeros(acc_v.shape, _F32)

        def pv_body(it, carry):
            m = m_v[...]
            l = l_v[...]
            acc = acc_v[...]
            for jj in range(_UNROLL):
                j = it * _UNROLL + jj
                p, l = exp_chunk(j, m, l)
                acc = pv_chunk(c, j, p, acc)
            l_v[...] = l
            acc_v[...] = acc
            for tt in range(nl // nit):
                t = it * (nl // nit) + tt
                uc_v[t] = conv_tile(c, t)
            return carry

        jax.lax.fori_loop(0, nit, pv_body, 0)
        uc = jnp.concatenate([uc_v[t] for t in range(nl)], axis=1)
        stage_out(c, acc_v[...], l_v[...], uc)


@jax.jit
def pallas_standalone__conformer_family_branchformer__speech_kernel(
    x: jax.Array,
    w_q: jax.Array,
    w_k: jax.Array,
    w_v: jax.Array,
    w_ao: jax.Array,
    w_up: jax.Array,
    dw: jax.Array,
    w_dn: jax.Array,
    w_merge: jax.Array,
):
    B, T, D = x.shape
    K = dw.shape[0]
    M, C = _BLK, _CHUNK
    assert T % M == 0 and D % _LANES == 0 and K // 2 <= _HALO and B == 2
    nblk = T // M
    total = B * nblk
    TP = pl.cdiv(T, C) * C
    TG = T + 2 * _HALO
    nl = D // _LANES

    def out_map(i):
        c = jnp.maximum(i - 1, 0)
        return (c // nblk, c % nblk, 0)

    vmem = pltpu.VMEM
    return pl.pallas_call(
        functools.partial(_kernel, B=B, T=T, D=D, K=K),
        grid=(total + 1,),
        in_specs=[pl.BlockSpec(memory_space=pl.ANY)] * 9,
        out_specs=pl.BlockSpec((1, M, D), out_map),
        out_shape=jax.ShapeDtypeStruct((B, T, D), x.dtype),
        scratch_shapes=[
            vmem((B * T, D), x.dtype),
            vmem((D, D), w_q.dtype), vmem((D, D), w_k.dtype), vmem((D, 2 * D), w_up.dtype),
            vmem((K, D), dw.dtype),
            vmem((8, D, D), _BF16),
            vmem((D, D), _BF16),
            vmem((nl, K, _LANES), _F32),
            vmem((B * TP, D), _BF16),
            vmem((nl, B * TG, _LANES), _F32),
            vmem((2, nl, M, _LANES), _F32),
            vmem((TP // C, M, C), _F32),
            vmem((M, _LANES), _F32),
            vmem((M, _LANES), _F32),
            vmem((M, D), _F32),
            vmem((nl, M, _LANES), _BF16),
            vmem((M, D), _BF16),
            pltpu.SMEM((TP // C,), jnp.int32),
            pltpu.SemaphoreType.DMA((10 + TP // C,)),
        ],
        compiler_params=pltpu.CompilerParams(
            dimension_semantics=("arbitrary",),
            vmem_limit_bytes=110 * 2**20,
        ),
    )(x.reshape(B * T, D), w_q, w_k, w_v, w_ao, w_up, dw, w_dn, w_merge)
```

```python
import functools
import math

import jax
import jax.numpy as jnp
import jax.experimental.pallas as pl
import jax.experimental.pallas.tpu as pltpu

_EPS = 1e-5
_LANES = 128
_BLK = 400
_CHUNK = 512
_HALO = 16
_GELU_C = math.sqrt(2.0 / math.pi)
_UNROLL = 4
_CONV_ROWS = 48
_FLAGS = None
_GATE = True

_F32 = jnp.float32
_BF16 = jnp.bfloat16
_U32 = jnp.uint32


def _dot(a, b):
    return jax.lax.dot_general(a, b, (((1,), (0,)), ((), ())), preferred_element_type=_F32)


def _dot_nt(a, b):
    return jax.lax.dot_general(a, b, (((1,), (1,)), ((), ())), preferred_element_type=_F32)


def _pack(x):
    return pltpu.bitcast(x.astype(_BF16), _U32)


def _unpack(w):
    return pltpu.bitcast(w, _BF16)


def _layernorm(x):
    m = jnp.mean(x, axis=-1, keepdims=True)
    xc = x - m
    v = jnp.mean(xc * xc, axis=-1, keepdims=True)
    return xc * jax.lax.rsqrt(v + _EPS)


def _gelu(x):
    inner = x * (_GELU_C + (_GELU_C * 0.044715) * (x * x))
    hx = 0.5 * x
    return hx + hx * jnp.tanh(inner)


def _tile(t):
    return slice(t * _LANES, (t + 1) * _LANES)


def _no_gate(x):
    return x


def _kernel(x_hbm, wq_hbm, wk_hbm, wv_hbm, wao_hbm, wup_hbm, dw_hbm, wdn_hbm, wm_hbm,
            o_ref,
            x_v, wq_v, wk_v, wupin_v, dw_v, w_v,
            a_v, wup_v, wo_v, dwf_v, xa_v, cv_v, gn_v, u_v, s_v, m_v, mx_v, l_v, acc_v, q_v, p_v, z_v,
            one_v, sems,
            *, B, T, D, K):
    M, C = _BLK, _CHUNK
    nblk = T // M
    total = B * nblk
    TP = pl.cdiv(T, C) * C
    nchunk = TP // C
    nl = D // _LANES
    nc = C // _LANES
    step = pl.program_id(0)

    def blk_pos(n):
        if isinstance(n, int):
            return n // nblk, (n % nblk) * M
        b = n // nblk
        return b, pl.multiple_of((n - b * nblk) * M, 16)

    def al(v, mult):
        return v if isinstance(v, int) else pl.multiple_of(v, mult)

    def xa_rows(r, rows):
        return pl.ds(al(r // 2, 8), rows // 2)

    def xq(n):
        b, r0 = blk_pos(n)
        return _unpack(xa_v[xa_rows(b * TP + r0, M), :])

    def q_tile(n, t):
        q = _dot(xq(n), _unpack(a_v[:, _tile(t)]))
        q_v[:, _tile(t)] = _pack(q)
        return q

    def g_tile(n, t):
        h = _dot(xq(n), _unpack(wup_v[:, _tile(nl + t)]))
        gn_v[t] = _gelu(h)
        return h

    def u_tile(n, t):
        h = _dot(xq(n), _unpack(wup_v[:, _tile(t)]))
        u_v[t] = _gelu(h)
        return h

    def qk_tile(n, j, t, mask):
        b, _ = blk_pos(n)
        k = _unpack(xa_v[xa_rows(b * TP + j * C + t * _LANES, _LANES), :])
        s = _dot_nt(_unpack(q_v[...]), k)
        if mask and t == nc - 1:
            col = jax.lax.broadcasted_iota(jnp.int32, s.shape, 1)
            s = jnp.where(col < T - j * C - t * _LANES, s, -jnp.inf)
        s_v[j, :, _tile(t)] = s
        return s

    def pv_tile(c, j, t, buf, first):
        b, _ = blk_pos(c)
        v = _unpack(xa_v[xa_rows(b * TP + j * C, C), _tile(t)])
        pv = _dot(_unpack(p_v[buf]), v)
        acc_v[t] = pv if first else acc_v[t] + pv
        return pv

    def out_tile(c, t):
        b, r0 = blk_pos(c)
        out = _dot(_unpack(z_v[...]), _unpack(wo_v[:, _tile(t)]))
        xr = x_v[pl.ds(al(b * T + r0, 16), M), _tile(t)].astype(_F32)
        o_ref[0, :, _tile(t)] = (xr + out).astype(o_ref.dtype)
        return out

    def norm_rows(b, r0, r, gate=_no_gate):
        xs = gate(x_v[pl.ds(al(b * T + r0 + r, 16), 16), :].astype(_F32))
        xa_v[xa_rows(b * TP + r0 + r, 16), :] = _pack(_layernorm(xs))

    def g_norm(r, gate=_no_gate):
        g = gate(jnp.concatenate([gn_v[t, r:r + 16, :] for t in range(nl)], axis=1))
        g = _layernorm(g)
        for t in range(nl):
            gn_v[t, r:r + 16, :] = g[:, _tile(t)]

    def max_rows(j, r, first, last, gate=_no_gate):
        cm = gate(s_v[j, r:r + 16, _tile(0)])
        if not first:
            cm = jnp.maximum(cm, mx_v[r:r + 16, :])
        for t in range(1, nc):
            cm = jnp.maximum(cm, s_v[j, r:r + 16, _tile(t)])
        if last:
            m_v[r:r + 16, :] = jnp.broadcast_to(jnp.max(cm, axis=-1, keepdims=True), cm.shape)
        else:
            mx_v[r:r + 16, :] = cm

    def exp_rows(j, buf, r, first, gate=_no_gate):
        m = gate(m_v[r:r + 16, :])
        l = None if first else l_v[r:r + 16, :]
        for t in range(nc):
            p = jnp.exp2(s_v[j, r:r + 16, _tile(t)] - m)
            l = p if l is None else l + p
            p_v[buf, r // 2:r // 2 + 8, _tile(t)] = _pack(p)
        l_v[r:r + 16, :] = l

    def scale_rows(r, gate=_no_gate):
        inv = 1.0 / jnp.sum(gate(l_v[r:r + 16, :]), axis=-1, keepdims=True)
        for t in range(nl):
            z_v[r // 2:r // 2 + 8, _tile(nl + t)] = _pack(acc_v[t, r:r + 16, :] * inv)

    def conv_piece(t, r, rows, gate=_no_gate):
        off = _HALO - K // 2
        conv = None
        for sh in range(8):
            taps = [i for i in range(K) if (off + i) % 8 == sh]
            span = (off + taps[-1]) // 8 * 8
            slab = cv_v[t, pl.ds(r + sh, rows + span), :]
            for i in taps:
                a = (off + i) // 8 * 8
                term = slab[a:a + rows] * jnp.tile(gate(dwf_v[t, i]), (rows // 8, 1))
                conv = term if conv is None else conv + term
        return _pack(u_v[t, pl.ds(r, rows), :] * conv)

    def conv_to_z(t, r, rows, gate=_no_gate):
        z_v[r // 2:(r + rows) // 2, _tile(t)] = conv_piece(t, r, rows, gate)

    def window_head(n):
        _, r0 = blk_pos(n)
        for t in range(nl):
            cv_v[t, _HALO + M:2 * _HALO + M, :] = jnp.where(r0 > 0, gn_v[t, :_HALO, :], 0.0)

    def advance_window(n, t):
        _, r0 = blk_pos(n)
        if isinstance(n, int):
            cv_v[t, :_HALO, :] = jnp.zeros((_HALO, _LANES), _F32)
        else:
            cv_v[t, :_HALO, :] = jnp.where(r0 > 0, cv_v[t, M:M + _HALO, :], 0.0)
        cv_v[t, _HALO:_HALO + M, :] = gn_v[t]

    rows16 = range(0, M, 16)
    conv_rows = [(r, min(_CONV_ROWS, M - r)) for r in range(0, M, _CONV_ROWS)]

    @pl.when(step == 0)
    @jax.named_scope("first")
    def _():
        def cp(src, dst, i):
            return pltpu.make_async_copy(src, dst, sems.at[i])

        def cx(j):
            r = al(j * C, C)
            return cp(x_hbm.at[pl.ds(r, C), :], x_v.at[pl.ds(r, C), :], 10 + j)

        c_wq, c_wk, c_wup = cp(wq_hbm, wq_v, 0), cp(wk_hbm, wk_v, 1), cp(wup_hbm, wupin_v, 2)
        c_w = [cp(wv_hbm, w_v.at[0], 3), cp(wao_hbm, w_v.at[3], 4), cp(wdn_hbm, w_v.at[1], 5),
               cp(wm_hbm.at[pl.ds(D, D), :], w_v.at[4], 6), cp(wm_hbm.at[pl.ds(0, D), :], w_v.at[5], 7)]
        c_dw = cp(dw_hbm, dw_v, 8)
        c_rest = cp(x_hbm.at[pl.ds(TP, B * T - TP), :], x_v.at[pl.ds(TP, B * T - TP), :], 9)
        for c in [c_wq, c_wk, cx(0), c_wup] + [cx(j) for j in range(1, nchunk)] + c_w + [c_dw, c_rest]:
            c.start()

        one_v[...] = jnp.ones(one_v.shape, jnp.int32)
        mx_v[...] = jnp.full(mx_v.shape, -jnp.inf, _F32)

        c_wq.wait()
        c_wk.wait()
        scale = float(D) ** -0.5 * math.log2(math.e)
        a_v[...] = _pack(_dot_nt(wq_v[...], wk_v[...]) * scale)
        cx(0).wait()
        for r in range(0, C, 16):
            norm_rows(0, 0, r)
        for t in range(nl):
            q_tile(0, t)
        c_wup.wait()
        wup_v[...] = pltpu.bitcast(wupin_v[...], _U32)
        for t in range(nl):
            g_tile(0, t)
        for t in range(nl):
            u_tile(0, t)
        for r in rows16:
            g_norm(r)
        for t in range(nl):
            advance_window(0, t)

        def qk_body(it, carry):
            for jj in range(_UNROLL):
                j = it * _UNROLL + jj
                if jj + 1 < _UNROLL:
                    cx(j + 1).wait()
                else:
                    pl.when(j + 1 < nchunk)(lambda: cx(j + 1).wait())
            for jj in range(_UNROLL):
                j = it * _UNROLL + jj
                for t in range(nc):
                    qk_tile(0, j, t, jj == _UNROLL - 1)
                for r in range(0, C, 16):
                    norm_rows(0, pl.multiple_of(jnp.minimum(j + 1, nchunk - 1) * C, C), r)
                for r in rows16:
                    max_rows(j, r, False, False)
            return carry

        jax.lax.fori_loop(0, nchunk // _UNROLL, qk_body, 0)
        m_v[...] = jnp.broadcast_to(jnp.max(mx_v[...], axis=-1, keepdims=True), m_v.shape)
        for b in range(B):
            xa_v[xa_rows(b * TP + T, TP - T), :] = jnp.zeros(((TP - T) // 2, D), _U32)
        for c in c_w:
            c.wait()

        def fold_body(i, carry):
            w_v[jnp.where(i == 0, 2, 8 - i)] = _dot(w_v[i], w_v[3 + i]).astype(_BF16)
            return carry

        jax.lax.fori_loop(0, 3, fold_body, 0)
        wo_v[:D // 2, :] = pltpu.bitcast(w_v[7], _U32)
        wo_v[D // 2:, :] = pltpu.bitcast(w_v[6], _U32)
        c_dw.wait()
        for t in range(nl):
            wt = dw_v[:, _tile(t)].astype(_F32)
            for i in range(K):
                dwf_v[t, i] = jnp.broadcast_to(wt[i:i + 1], (8, _LANES))
        c_rest.wait()
        for b in range(1, B):
            for r in rows16:
                norm_rows(b, 0, r)

    @pl.when(jnp.logical_and(step > 0, step < total))
    @jax.named_scope("main")
    def _():
        n, c = step, step - 1
        P = functools.partial
        keep = one_v[...] != 0

        tasks = {}
        order = []

        def add(name, fns):
            tasks[name] = []
            for f in fns:
                tasks[name].append(len(order))
                order.append((f, []))

        add("q", [P(q_tile, n, t) for t in range(nl)])
        add(("pv", 0), [P(pv_tile, c, 0, t, 0, True) for t in range(nl)])
        add("g", [P(g_tile, n, t) for t in range(nl)])
        for j in range(nchunk):
            add(("qk", j), [P(qk_tile, n, j, t, j == nchunk - 1) for t in range(nc)])
            if j + 1 < nchunk:
                add(("pv", j + 1), [P(pv_tile, c, j + 1, t, (j + 1) % 2, False) for t in range(nl)])
        add("u", [P(u_tile, n, t) for t in range(nl)])
        add("out", [P(out_tile, c, t) for t in range(nl)])

        def spread(fns, *names):
            slots = [i for name in names for i in tasks[name]]
            per = M // 8
            for k, f in enumerate(fns):
                pos = k * len(slots) * per // len(fns)
                order[slots[pos // per]][1].append((pos % per, f))

        last = nchunk - 1
        spread([P(exp_rows, 1, 1, r, False) for r in rows16], ("pv", 0), ("qk", 0))
        for j in range(1, last):
            spread([P(exp_rows, j + 1, (j + 1) % 2, r, False) for r in rows16], ("pv", j), ("qk", j))
        for j in range(last):
            spread([P(max_rows, j, r, j == 0, False) for r in rows16], ("pv", j + 1))
        spread([P(g_norm, r) for r in rows16[:1]] + [lambda gate: window_head(n)]
               + [P(g_norm, r) for r in rows16[1:]], ("qk", 0), ("pv", 1))
        spread([P(conv_to_z, t, r, rows) for r, rows in conv_rows for t in range(nl)],
               *[(name, j + d) for j in range(1, last) for name, d in (("qk", 0), ("pv", 1))])
        spread([P(scale_rows, r) for r in rows16], ("qk", last))
        spread([P(max_rows, last, r, False, True) for r in rows16], "u")
        nxt = pl.multiple_of(jnp.minimum(step, nblk - 1) * M, 16)
        spread([P(norm_rows, b, nxt, r) for b in range(1, B) for r in rows16], "out")

        for r in rows16:
            exp_rows(0, 0, r, True)
        for f, fillers in order:
            res = f()
            for pos, filler in sorted(fillers, key=lambda e: e[0]):
                def gate(x, g=res[8 * pos:8 * pos + 8]):
                    reps = (x.shape[0] // 8, x.shape[1] // _LANES)
                    return jnp.where(jnp.tile(keep, reps), x, jnp.tile(g, reps))
                filler(gate=gate if _GATE else _no_gate)
        for t in range(nl):
            advance_window(n, t)

    @pl.when(step == total)
    @jax.named_scope("last")
    def _():
        c = total - 1
        nit = nchunk // _UNROLL
        for t in range(nl):
            cv_v[t, _HALO + M:2 * _HALO + M, :] = jnp.zeros((_HALO, _LANES), _F32)
        l_v[...] = jnp.zeros(l_v.shape, _F32)
        acc_v[...] = jnp.zeros(acc_v.shape, _F32)

        def pv_body(it, carry):
            for jj in range(_UNROLL):
                j = it * _UNROLL + jj
                for r in rows16:
                    exp_rows(j, jj % 2, r, False)
                for t in range(nl):
                    pv_tile(c, j, t, jj % 2, False)
            for tt in range(nl // nit):
                t = it * (nl // nit) + tt
                for r, rows in conv_rows:
                    gn_v[t, r // 2:(r + rows) // 2, :] = pltpu.bitcast(conv_piece(t, r, rows), _F32)
            return carry

        jax.lax.fori_loop(0, nit, pv_body, 0)
        for t in range(nl):
            z_v[:, _tile(t)] = pltpu.bitcast(gn_v[t, :M // 2, :], _U32)
        for r in rows16:
            scale_rows(r)
        for t in range(nl):
            out_tile(c, t)


@jax.jit
def pallas_standalone__conformer_family_branchformer__speech_kernel(
    x: jax.Array,
    w_q: jax.Array,
    w_k: jax.Array,
    w_v: jax.Array,
    w_ao: jax.Array,
    w_up: jax.Array,
    dw: jax.Array,
    w_dn: jax.Array,
    w_merge: jax.Array,
):
    B, T, D = x.shape
    K = dw.shape[0]
    M, C = _BLK, _CHUNK
    assert T % M == 0 and D % _LANES == 0 and K // 2 <= _HALO and B == 2
    nblk = T // M
    total = B * nblk
    TP = pl.cdiv(T, C) * C
    nl = D // _LANES

    def out_map(i):
        c = jnp.maximum(i - 1, 0)
        return (c // nblk, c % nblk, 0)

    vmem = pltpu.VMEM
    return pl.pallas_call(
        functools.partial(_kernel, B=B, T=T, D=D, K=K),
        grid=(total + 1,),
        in_specs=[pl.BlockSpec(memory_space=pl.ANY)] * 9,
        out_specs=pl.BlockSpec((1, M, D), out_map),
        out_shape=jax.ShapeDtypeStruct((B, T, D), x.dtype),
        scratch_shapes=[
            vmem((B * T, D), x.dtype),
            vmem((D, D), w_q.dtype), vmem((D, D), w_k.dtype), vmem((D, 2 * D), w_up.dtype),
            vmem((K, D), dw.dtype),
            vmem((8, D, D), _BF16),
            vmem((D // 2, D), _U32),
            vmem((D // 2, 2 * D), _U32),
            vmem((D, D), _U32),
            vmem((nl, K, 8, _LANES), _F32),
            vmem((B * TP // 2, D), _U32),
            vmem((nl, M + 2 * _HALO, _LANES), _F32),
            vmem((nl, M, _LANES), _F32),
            vmem((nl, M, _LANES), _F32),
            vmem((TP // C, M, C), _F32),
            vmem((M, _LANES), _F32),
            vmem((M, _LANES), _F32),
            vmem((M, _LANES), _F32),
            vmem((nl, M, _LANES), _F32),
            vmem((M // 2, D), _U32),
            vmem((2, M // 2, C), _U32),
            vmem((M // 2, 2 * D), _U32),
            vmem((8, _LANES), jnp.int32),
            pltpu.SemaphoreType.DMA((10 + TP // C,)),
        ],
        compiler_params=pltpu.CompilerParams(
            dimension_semantics=("arbitrary",),
            vmem_limit_bytes=110 * 2**20,
            flags=_FLAGS,
        ),
    )(x.reshape(B * T, D), w_q, w_k, w_v, w_ao, w_up, dw, w_dn, w_merge)
```

```python
import functools
import math

import jax
import jax.numpy as jnp
import jax.experimental.pallas as pl
import jax.experimental.pallas.tpu as pltpu

_EPS = 1e-5
_LANES = 128
_BLK = 400
_CHUNK = 512
_HALO = 16
_GELU_C = math.sqrt(2.0 / math.pi)
_UNROLL = 4
_CONV_ROWS = 48
_CONV_FROM = 1
_CONV_TO = 6
_FLAGS = None
_NORM_AT = (("pv", 0), "g")

_F32 = jnp.float32
_BF16 = jnp.bfloat16
_U32 = jnp.uint32


def _dot(a, b):
    return jax.lax.dot_general(a, b, (((1,), (0,)), ((), ())), preferred_element_type=_F32)


def _dot_nt(a, b):
    return jax.lax.dot_general(a, b, (((1,), (1,)), ((), ())), preferred_element_type=_F32)


def _pack(x):
    return pltpu.bitcast(x.astype(_BF16), _U32)


def _unpack(w):
    return pltpu.bitcast(w, _BF16)


def _layernorm(x):
    m = jnp.mean(x, axis=-1, keepdims=True)
    xc = x - m
    v = jnp.mean(xc * xc, axis=-1, keepdims=True)
    return xc * jax.lax.rsqrt(v + _EPS)


def _gelu(x):
    inner = x * (_GELU_C + (_GELU_C * 0.044715) * (x * x))
    hx = 0.5 * x
    return hx + hx * jnp.tanh(inner)


def _tile(t):
    return slice(t * _LANES, (t + 1) * _LANES)


def _no_gate(x):
    return x


def _norm_rows_per_step(T):
    return pl.cdiv(T, 16 * (T // _BLK - 1)) * 16


def _kernel(x_hbm, wq_hbm, wk_hbm, wv_hbm, wao_hbm, wup_hbm, dw_hbm, wdn_hbm, wm_hbm,
            o_ref,
            x_v, wq_v, wk_v, wupin_v, dw_v, wv_v, wao_v, wdn_v, wm_v, wvo_v, st_v, xq_v,
            a_v, wup_v, wo_v, dwf_v, xa_v, cv_v, gn_v, u_v, s_v, m_v, mx_v, l_v, acc_v, q_v, p_v, z_v,
            one_v, sems,
            *, B, T, D, K):
    M, C = _BLK, _CHUNK
    nblk = T // M
    total = B * nblk
    TP = pl.cdiv(T, C) * C
    nchunk = TP // C
    nl = D // _LANES
    nc = C // _LANES
    NR = _norm_rows_per_step(T)
    step = pl.program_id(0)

    def blk_pos(n):
        if isinstance(n, int):
            return n // nblk, (n % nblk) * M
        b = n // nblk
        return b, pl.multiple_of((n - b * nblk) * M, 16)

    def al(v, mult):
        return v if isinstance(v, int) else pl.multiple_of(v, mult)

    def xa_rows(r, rows):
        return pl.ds(al(r // 2, 8), rows // 2)

    def select_rows(n):
        b, r0 = blk_pos(n)
        xq_v[...] = xa_v[xa_rows(b * TP + r0, M), :]

    def xq():
        return _unpack(xq_v[...])

    def q_tile(n, t):
        q = _dot(xq(), _unpack(a_v[:, _tile(t)]))
        q_v[:, _tile(t)] = _pack(q)
        return q

    def g_tile(n, t):
        h = _dot(xq(), _unpack(wup_v[:, _tile(nl + t)]))
        gn_v[t] = _gelu(h)
        return h

    def u_tile(n, t):
        h = _dot(xq(), _unpack(wup_v[:, _tile(t)]))
        u_v[t] = _gelu(h)
        return h

    def copy_rows(slot, dst0, rows):
        xa_v[pl.ds(al(dst0, 8), rows), :] = st_v[slot, :rows, :]

    def qk_tile(n, j, t, mask, track_max):
        b, _ = blk_pos(n)
        k = _unpack(xa_v[xa_rows(b * TP + j * C + t * _LANES, _LANES), :])
        s = _dot_nt(_unpack(q_v[...]), k)
        if mask and t == nc - 1:
            col = jax.lax.broadcasted_iota(jnp.int32, s.shape, 1)
            s = jnp.where(col < T - j * C - t * _LANES, s, -jnp.inf)
        s_v[j, :, _tile(t)] = s
        if track_max:
            mx_v[...] = jnp.maximum(mx_v[...], s)
        return s

    def pv_tile(c, j, t, buf, first):
        b, _ = blk_pos(c)
        v = _unpack(xa_v[xa_rows(b * TP + j * C, C), _tile(t)])
        pv = _dot(_unpack(p_v[buf]), v)
        acc_v[t] = pv if first else acc_v[t] + pv
        return pv

    def out_tile(c, t):
        b, r0 = blk_pos(c)
        out = _dot(_unpack(z_v[...]), _unpack(wo_v[:, _tile(t)]))
        xr = x_v[pl.ds(al(b * T + r0, 16), M), _tile(t)].astype(_F32)
        o_ref[0, :, _tile(t)] = (xr + out).astype(o_ref.dtype)
        return out

    def norm_rows(src0, dst_ref, dst0, r, gate=_no_gate):
        xs = gate(x_v[pl.ds(al(src0 + r, 16), 16), :].astype(_F32))
        dst_ref[pl.ds(al(dst0 + r // 2, 8), 8), :] = _pack(_layernorm(xs))

    def g_norm(r, gate=_no_gate):
        g = gate(jnp.concatenate([gn_v[t, r:r + 16, :] for t in range(nl)], axis=1))
        g = _layernorm(g)
        for t in range(nl):
            gn_v[t, r:r + 16, :] = g[:, _tile(t)]

    def max_rows(j, r, first, last, gate=_no_gate):
        cm = gate(s_v[j, r:r + 16, _tile(0)])
        if not first:
            cm = jnp.maximum(cm, mx_v[r:r + 16, :])
        for t in range(1, nc):
            cm = jnp.maximum(cm, s_v[j, r:r + 16, _tile(t)])
        if last:
            m_v[r:r + 16, :] = jnp.broadcast_to(jnp.max(cm, axis=-1, keepdims=True), cm.shape)
        else:
            mx_v[r:r + 16, :] = cm

    def exp_rows(j, buf, r, first, gate=_no_gate):
        m = gate(m_v[r:r + 16, :])
        l = None if first else l_v[r:r + 16, :]
        for t in range(nc):
            p = jnp.exp2(s_v[j, r:r + 16, _tile(t)] - m)
            l = p if l is None else l + p
            p_v[buf, r // 2:r // 2 + 8, _tile(t)] = _pack(p)
        l_v[r:r + 16, :] = l

    def scale_rows(r, gate=_no_gate):
        inv = 1.0 / jnp.sum(gate(l_v[r:r + 16, :]), axis=-1, keepdims=True)
        for t in range(nl):
            z_v[r // 2:r // 2 + 8, _tile(nl + t)] = _pack(acc_v[t, r:r + 16, :] * inv)

    def conv_piece(t, r, rows, gate=_no_gate):
        off = _HALO - K // 2
        conv = None
        for sh in range(8):
            taps = [i for i in range(K) if (off + i) % 8 == sh]
            span = (off + taps[-1]) // 8 * 8
            slab = cv_v[t, pl.ds(r + sh, rows + span), :]
            for i in taps:
                a = (off + i) // 8 * 8
                term = slab[a:a + rows] * jnp.tile(gate(dwf_v[t, i]), (rows // 8, 1))
                conv = term if conv is None else conv + term
        return _pack(u_v[t, pl.ds(r, rows), :] * conv)

    def conv_to_z(t, r, rows, gate=_no_gate):
        z_v[r // 2:(r + rows) // 2, _tile(t)] = conv_piece(t, r, rows, gate)

    def window_head(n):
        _, r0 = blk_pos(n)
        for t in range(nl):
            cv_v[t, _HALO + M:2 * _HALO + M, :] = jnp.where(r0 > 0, gn_v[t, :_HALO, :], 0.0)

    def advance_window(n, t):
        _, r0 = blk_pos(n)
        if isinstance(n, int):
            cv_v[t, :_HALO, :] = jnp.zeros((_HALO, _LANES), _F32)
        else:
            cv_v[t, :_HALO, :] = jnp.where(r0 > 0, cv_v[t, M:M + _HALO, :], 0.0)
        cv_v[t, _HALO:_HALO + M, :] = gn_v[t]

    class Plan:
        def __init__(self):
            self.order, self.slots = [], {}

        def add(self, name, fns):
            self.slots[name] = list(range(len(self.order), len(self.order) + len(fns)))
            self.order += [(f, []) for f in fns]

        def spread(self, fns, *names, skip=0):
            slots = [i for name in names for i in self.slots[name]]
            slots = slots[:len(slots) - skip]
            for k, f in enumerate(fns):
                pos = k * len(slots) / len(fns)
                self.order[slots[int(pos)]][1].append((pos - int(pos), f))

        def run(self):
            keep = one_v[...] != 0
            for f, fillers in self.order:
                res = f()
                for frac, filler in sorted(fillers, key=lambda e: e[0]):
                    r = int(frac * (res.shape[0] // 8)) * 8

                    def gate(x, g=res[r:r + 8, :_LANES]):
                        reps = (x.shape[0] // 8, x.shape[1] // _LANES)
                        return jnp.where(jnp.tile(keep, reps), x, jnp.tile(g, reps))

                    filler(gate=gate)

    P = functools.partial
    rows16 = range(0, M, 16)
    conv_rows = [(r, min(_CONV_ROWS, M - r)) for r in range(0, M, _CONV_ROWS)]

    @pl.when(step == 0)
    @jax.named_scope("first")
    def _():
        def cp(src, dst, i):
            return pltpu.make_async_copy(src, dst, sems.at[i])

        def cx(j):
            r = al(j * C, C)
            return cp(x_hbm.at[pl.ds(r, C), :], x_v.at[pl.ds(r, C), :], 10 + j)

        c_wq, c_wk, c_wup = cp(wq_hbm, wq_v, 0), cp(wk_hbm, wk_v, 1), cp(wup_hbm, wupin_v, 2)
        c_w = [cp(wv_hbm, wv_v, 3), cp(wao_hbm, wao_v, 4), cp(wdn_hbm, wdn_v, 5), cp(wm_hbm, wm_v, 6)]
        c_dw = cp(dw_hbm, dw_v, 8)
        c_rest = cp(x_hbm.at[pl.ds(TP, B * T - TP), :], x_v.at[pl.ds(TP, B * T - TP), :], 9)
        for c in [c_wq, c_wk, cx(0), c_wup] + [cx(j) for j in range(1, nchunk)] + c_w + [c_dw, c_rest]:
            c.start()

        one_v[...] = jnp.ones(one_v.shape, jnp.int32)
        mx_v[...] = jnp.full(mx_v.shape, -jnp.inf, _F32)

        def a_tile(t):
            a = _dot_nt(wq_v[...], wk_v[_tile(t), :])
            a_v[:, _tile(t)] = _pack(a * (float(D) ** -0.5 * math.log2(math.e)))
            return a

        c_wq.wait()
        c_wk.wait()
        cx(0).wait()
        plan = Plan()
        plan.add("a", [P(a_tile, t) for t in range(nl)])
        plan.spread([P(norm_rows, 0, xa_v, 0, r) for r in range(0, C, 16)], "a", skip=2)
        plan.run()
        select_rows(0)
        c_wup.wait()
        cx(1).wait()
        wup_v[...] = pltpu.bitcast(wupin_v[...], _U32)
        plan = Plan()
        plan.add("g", [P(g_tile, 0, t) for t in range(nl)])
        plan.add("q", [P(q_tile, 0, t) for t in range(nl)])
        plan.add("u", [P(u_tile, 0, t) for t in range(nl)])
        plan.spread([P(g_norm, r) for r in rows16], "q")
        plan.spread([P(norm_rows, C, st_v.at[_UNROLL - 1], 0, r) for r in range(0, C, 16)], "g", "u", skip=1)
        plan.run()
        for t in range(nl):
            advance_window(0, t)

        def qk_body(it, carry):
            for jj in range(_UNROLL):
                j = it * _UNROLL + jj
                if jj + 2 < _UNROLL:
                    cx(j + 2).wait()
                else:
                    pl.when(j + 2 < nchunk)(lambda: cx(j + 2).wait())
            plan = Plan()
            for jj in range(_UNROLL):
                j = it * _UNROLL + jj
                plan.add(jj, [P(qk_tile, 0, j, t, jj == _UNROLL - 1, True) for t in range(nc)])
                plan.spread([P(norm_rows, jnp.minimum(j + 2, nchunk - 1) * C, st_v.at[jj], 0, r)
                             for r in range(0, C, 16)], jj)
                plan.add((jj, "copy"), [P(copy_rows, (jj - 1) % _UNROLL,
                                          jnp.minimum(j + 1, nchunk - 1) * (C // 2), C // 2)])
            plan.run()
            return carry

        jax.lax.fori_loop(0, nchunk // _UNROLL, qk_body, 0)
        for c in c_w + [c_dw, c_rest]:
            c.wait()

        def fold_tile(lhs, rhs_rows, dst, t):
            w = _dot(lhs[...], wm_v[rhs_rows, _tile(t)] if rhs_rows is not None else wao_v[:, _tile(t)])
            dst(t, w)
            return w

        def to_wvo(t, w):
            wvo_v[:, _tile(t)] = w.astype(_BF16)

        def to_wo(half, t, w):
            wo_v[half * D // 2:(half + 1) * D // 2, _tile(t)] = _pack(w)

        def taps(t, gate):
            wt = dw_v[:, _tile(t)].astype(_F32)
            for i in range(K):
                dwf_v[t, i] = jnp.broadcast_to(wt[i:i + 1], (8, _LANES))

        def finish_max(r, gate):
            cm = gate(mx_v[r:r + 16, :])
            m_v[r:r + 16, :] = jnp.broadcast_to(jnp.max(cm, axis=-1, keepdims=True), cm.shape)

        plan = Plan()
        plan.add("vo", [P(fold_tile, wv_v, None, to_wvo, t) for t in range(nl)])
        plan.add("dm", [P(fold_tile, wdn_v, slice(D, 2 * D), P(to_wo, 0), t) for t in range(nl)])
        plan.add("vom", [P(fold_tile, wvo_v, slice(0, D), P(to_wo, 1), t) for t in range(nl)])
        plan.spread([P(finish_max, r) for r in rows16], "vo")
        plan.spread([P(taps, t) for t in range(nl)], "dm")
        plan.run()
        for b in range(B):
            xa_v[xa_rows(b * TP + T, TP - T), :] = jnp.zeros(((TP - T) // 2, D), _U32)
        select_rows(1)

    @pl.when(jnp.logical_and(step > 0, step < total))
    @jax.named_scope("main")
    def _():
        n, c = step, step - 1
        last = nchunk - 1
        plan = Plan()
        plan.add("q", [P(q_tile, n, t) for t in range(nl)])
        plan.add(("pv", 0), [P(pv_tile, c, 0, t, 0, True) for t in range(nl)])
        plan.add("g", [P(g_tile, n, t) for t in range(nl)])
        for j in range(nchunk):
            plan.add(("qk", j), [P(qk_tile, n, j, t, j == last, False) for t in range(nc)])
            if j < last:
                plan.add(("pv", j + 1), [P(pv_tile, c, j + 1, t, (j + 1) % 2, False) for t in range(nl)])
        plan.add("u", [P(u_tile, n, t) for t in range(nl)])
        plan.add("out", [P(out_tile, c, t) for t in range(nl)])

        for j in range(last):
            plan.spread([P(exp_rows, j + 1, (j + 1) % 2, r, False) for r in rows16], ("pv", j), ("qk", j))
            plan.spread([P(max_rows, j, r, j == 0, False) for r in rows16], ("pv", j + 1))
        plan.spread([P(g_norm, r) for r in rows16[:1]] + [lambda gate: window_head(n)]
                    + [P(g_norm, r) for r in rows16[1:]], ("qk", 0), ("pv", 1))
        plan.spread([P(conv_to_z, t, r, rows) for r, rows in conv_rows for t in range(nl)],
                    *[(name, j + d) for j in range(_CONV_FROM, _CONV_TO) for name, d in (("qk", 0), ("pv", 1))])
        plan.spread([P(scale_rows, r) for r in rows16], ("qk", last))
        plan.spread([P(max_rows, last, r, False, True) for r in rows16], "out", skip=1)
        def piece(i):
            return jnp.clip(i * (NR // 2), 0, (T - NR) // 2)

        copy_rows(0, TP // 2 + piece(c - 1), NR // 2)
        plan.spread([P(norm_rows, T + 2 * piece(c), st_v.at[0], 0, r) for r in range(0, NR, 16)], *_NORM_AT)

        for r in rows16:
            exp_rows(0, 0, r, True)
        plan.run()
        select_rows(jnp.minimum(n + 1, total - 1))
        for t in range(nl):
            advance_window(n, t)

    @pl.when(step == total)
    @jax.named_scope("last")
    def _():
        c = total - 1
        nit = nchunk // _UNROLL
        for t in range(nl):
            cv_v[t, _HALO + M:2 * _HALO + M, :] = jnp.zeros((_HALO, _LANES), _F32)
        l_v[...] = jnp.zeros(l_v.shape, _F32)
        acc_v[...] = jnp.zeros(acc_v.shape, _F32)

        def conv_to_st(t, r, rows, gate):
            gn_v[t, r // 2:(r + rows) // 2, :] = pltpu.bitcast(conv_piece(t, r, rows, gate), _F32)

        def pv_body(it, carry):
            plan = Plan()
            for jj in range(_UNROLL):
                j = it * _UNROLL + jj
                plan.add(jj, [P(pv_tile, c, j, t, jj % 2, False) for t in range(nl)])
                if jj + 1 < _UNROLL:
                    plan.spread([P(exp_rows, j + 1, (jj + 1) % 2, r, False) for r in rows16], jj, skip=1)
            plan.spread([P(conv_to_st, it * (nl // nit) + tt, r, rows)
                         for tt in range(nl // nit) for r, rows in conv_rows], *range(_UNROLL), skip=1)
            for r in rows16:
                exp_rows(it * _UNROLL, 0, r, False)
            plan.run()
            return carry

        jax.lax.fori_loop(0, nit, pv_body, 0)
        for t in range(nl):
            z_v[:, _tile(t)] = pltpu.bitcast(gn_v[t, :M // 2, :], _U32)
        for r in rows16:
            scale_rows(r)
        for t in range(nl):
            out_tile(c, t)


@jax.jit
def pallas_standalone__conformer_family_branchformer__speech_kernel(
    x: jax.Array,
    w_q: jax.Array,
    w_k: jax.Array,
    w_v: jax.Array,
    w_ao: jax.Array,
    w_up: jax.Array,
    dw: jax.Array,
    w_dn: jax.Array,
    w_merge: jax.Array,
):
    B, T, D = x.shape
    K = dw.shape[0]
    M, C = _BLK, _CHUNK
    assert T % M == 0 and D % _LANES == 0 and K // 2 <= _HALO and B == 2
    nblk = T // M
    total = B * nblk
    TP = pl.cdiv(T, C) * C
    nl = D // _LANES
    NR = _norm_rows_per_step(T)

    def out_map(i):
        c = jnp.maximum(i - 1, 0)
        return (c // nblk, c % nblk, 0)

    vmem = pltpu.VMEM
    return pl.pallas_call(
        functools.partial(_kernel, B=B, T=T, D=D, K=K),
        grid=(total + 1,),
        in_specs=[pl.BlockSpec(memory_space=pl.ANY)] * 9,
        out_specs=pl.BlockSpec((1, M, D), out_map),
        out_shape=jax.ShapeDtypeStruct((B, T, D), x.dtype),
        scratch_shapes=[
            vmem((B * T, D), x.dtype),
            vmem((D, D), w_q.dtype), vmem((D, D), w_k.dtype), vmem((D, 2 * D), w_up.dtype),
            vmem((K, D), dw.dtype),
            vmem((D, D), w_v.dtype), vmem((D, D), w_ao.dtype), vmem((D, D), w_dn.dtype),
            vmem((2 * D, D), w_merge.dtype),
            vmem((D, D), _BF16),
            vmem((_UNROLL, max(C, NR) // 2, D), _U32),
            vmem((M // 2, D), _U32),
            vmem((D // 2, D), _U32),
            vmem((D // 2, 2 * D), _U32),
            vmem((D, D), _U32),
            vmem((nl, K, 8, _LANES), _F32),
            vmem((B * TP // 2, D), _U32),
            vmem((nl, M + 2 * _HALO, _LANES), _F32),
            vmem((nl, M, _LANES), _F32),
            vmem((nl, M, _LANES), _F32),
            vmem((TP // C, M, C), _F32),
            vmem((M, _LANES), _F32),
            vmem((M, _LANES), _F32),
            vmem((M, _LANES), _F32),
            vmem((nl, M, _LANES), _F32),
            vmem((M // 2, D), _U32),
            vmem((2, M // 2, C), _U32),
            vmem((M // 2, 2 * D), _U32),
            vmem((8, _LANES), jnp.int32),
            pltpu.SemaphoreType.DMA((10 + TP // C,)),
        ],
        compiler_params=pltpu.CompilerParams(
            dimension_semantics=("arbitrary",),
            vmem_limit_bytes=110 * 2**20,
            flags=_FLAGS,
        ),
    )(x.reshape(B * T, D), w_q, w_k, w_v, w_ao, w_up, dw, w_dn, w_merge)
```

```python
import functools
import math

import jax
import jax.numpy as jnp
import jax.experimental.pallas as pl
import jax.experimental.pallas.tpu as pltpu

_EPS = 1e-5
_LANES = 128
_BLK = 400
_CHUNK = 512
_HALO = 16
_GELU_C = math.sqrt(2.0 / math.pi)
_UNROLL = 4
_CONV_ROWS = 48
_CONV_ROWS_LAST = 16
_QK_SKIP = 1
_E1 = True
_E2 = False
_CUTS = (0, 14, 20, 26, 32, 38, 44, 50)
_TSKIP = 0
_LAG = 2
_TAIL_AT = ("q", ("pv", 0), "g", ("qk", 0), ("pv", 1), ("qk", 1), ("pv", 2), ("qk", 2), ("pv", 3), ("qk", 3), ("pv", 4), ("qk", 4), ("pv", 5), ("qk", 5))
_CONV_FROM = 1
_CONV_TO = 6
_FLAGS = None
_NORM_AT = (("pv", 0), "g")

_F32 = jnp.float32
_BF16 = jnp.bfloat16
_U32 = jnp.uint32


def _dot(a, b):
    return jax.lax.dot_general(a, b, (((1,), (0,)), ((), ())), preferred_element_type=_F32)


def _dot_nt(a, b):
    return jax.lax.dot_general(a, b, (((1,), (1,)), ((), ())), preferred_element_type=_F32)


def _pack(x):
    return pltpu.bitcast(x.astype(_BF16), _U32)


def _unpack(w):
    return pltpu.bitcast(w, _BF16)


def _layernorm(x):
    m = jnp.mean(x, axis=-1, keepdims=True)
    xc = x - m
    v = jnp.mean(xc * xc, axis=-1, keepdims=True)
    return xc * jax.lax.rsqrt(v + _EPS)


def _gelu(x):
    inner = x * (_GELU_C + (_GELU_C * 0.044715) * (x * x))
    hx = 0.5 * x
    return hx + hx * jnp.tanh(inner)


def _tile(t):
    return slice(t * _LANES, (t + 1) * _LANES)


def _no_gate(x):
    return x


def _norm_rows_per_step(T):
    return pl.cdiv(T, 16 * (T // _BLK - 1)) * 16


def _kernel(x_hbm, wq_hbm, wk_hbm, wv_hbm, wao_hbm, wup_hbm, dw_hbm, wdn_hbm, wm_hbm,
            o_hbm,
            x_v, wq_v, wk_v, wupin_v, dw_v, wv_v, wao_v, wdn_v, wm_v, wvo_v, st_v, xq_v,
            a_v, wup_v, wo_v, dwf_v, xa_v, cv_v, gn_v, u_v, s_v, m_v, mx_v, l_v, acc_v, q_v, p_v, z_v,
            one_v, vt_v, lt_v, acct_v, ob_v, sems, out_sems,
            *, B, T, D, K):
    M, C = _BLK, _CHUNK
    nblk = T // M
    total = B * nblk
    TP = pl.cdiv(T, C) * C
    nchunk = TP // C
    nl = D // _LANES
    nc = C // _LANES
    TAIL = T % _LANES
    NR = _norm_rows_per_step(T)

    def blk_pos(n):
        if isinstance(n, int):
            return n // nblk, (n % nblk) * M
        b = n // nblk
        return b, pl.multiple_of((n - b * nblk) * M, 16)

    def al(v, mult):
        return v if isinstance(v, int) else pl.multiple_of(v, mult)

    def xa_rows(r, rows):
        return pl.ds(al(r // 2, 8), rows // 2)

    def select_rows(n):
        b, r0 = blk_pos(n)
        xq_v[...] = xa_v[xa_rows(b * TP + r0, M), :]

    def xq():
        return _unpack(xq_v[...])

    def q_tile(n, t):
        q = _dot(xq(), _unpack(a_v[:, _tile(t)]))
        q_v[:, _tile(t)] = _pack(q)
        return q

    def g_tile(n, t):
        h = _dot(xq(), _unpack(wup_v[:, _tile(nl + t)]))
        gn_v[t] = _gelu(h)
        return h

    def u_tile(n, t):
        h = _dot(xq(), _unpack(wup_v[:, _tile(t)]))
        u_v[t] = _gelu(h)
        return h

    def copy_rows(dst0, rows):
        xa_v[pl.ds(al(dst0, 8), rows), :] = st_v[...]

    def qk_tile(n, j, t, mask, track_max):
        b, _ = blk_pos(n)
        k = _unpack(xa_v[xa_rows(b * TP + j * C + t * _LANES, _LANES), :])
        s = _dot_nt(_unpack(q_v[...]), k)
        if mask and t == nc - 1:
            col = jax.lax.broadcasted_iota(jnp.int32, s.shape, 1)
            s = jnp.where(col < T - j * C - t * _LANES, s, -jnp.inf)
        s_v[j, :, _tile(t)] = s
        if track_max:
            mx_v[...] = jnp.maximum(mx_v[...], s)
        return s

    def qk_tail(n, i):
        b, _ = blk_pos(n)
        r, rows = i * _LANES, min(_LANES, M - i * _LANES)
        q = _unpack(q_v[r // 2:(r + rows) // 2, :])
        if rows == _LANES:
            s = _dot_nt(_unpack(xa_v[xa_rows(b * TP + T - TAIL, TAIL), :]), q)
            pad = jnp.full((_LANES - TAIL, _LANES), -jnp.inf, _F32)
            s = jnp.concatenate([s, pad], axis=0).T
        else:
            s = _dot_nt(q, _unpack(xa_v[xa_rows(b * TP + T - TAIL, _LANES), :]))
            col = jax.lax.broadcasted_iota(jnp.int32, s.shape, 1)
            s = jnp.where(col < TAIL, s, -jnp.inf)
        s_v[nchunk - 1, r:r + rows, _tile(nc - 1)] = s
        return s

    def tail_values(c):
        b, _ = blk_pos(c)
        v = _unpack(xa_v[xa_rows(b * TP + T - TAIL, TAIL), :]).astype(_F32)
        for k in range(TAIL):
            for t in range(nl):
                vt_v[k, t] = jnp.broadcast_to(v[k:k + 1, _tile(t)], (8, _LANES))

    def pv_tail(r, gate=_no_gate):
        p = jnp.exp2(s_v[nchunk - 1, r:r + 8, _tile(nc - 1)] - gate(m_v[r:r + 8, :]))
        lt_v[r:r + 8, :] = p
        acc = [None] * nl
        done = []
        keep = one_v[...] != 0
        for k in range(TAIL):
            if k >= _LAG:
                p = jnp.where(keep, p, done[k - _LAG])
            pk = jnp.broadcast_to(p[:, k:k + 1], (8, _LANES))
            for t in range(nl):
                term = pk * vt_v[k, t]
                acc[t] = term if k == 0 else acc[t] + term
            done.append(acc[k % nl])
        for t in range(nl):
            acct_v[t, r:r + 8, :] = acc[t]

    def pv_tile(c, j, t, buf, first, keys=C, tail_rows=None):
        b, _ = blk_pos(c)
        v = _unpack(xa_v[xa_rows(b * TP + j * C, keys), _tile(t)])
        pv = _dot(_unpack(p_v[buf * M // 2:(buf + 1) * M // 2, :keys]), v)
        acc = pv if first else acc_v[t] + pv
        if tail_rows is None:
            acc_v[t] = acc
        else:
            lo, hi = tail_rows
            if lo > 0:
                acc_v[t, :lo, :] = acc[:lo]
            acc_v[t, lo:hi, :] = acc[lo:hi] + acct_v[t, lo:hi, :]
            if hi < M:
                acc_v[t, hi:, :] = acc[hi:]
        return pv

    def out_tile(c, t):
        b, r0 = blk_pos(c)
        out = _dot(_unpack(z_v[...]), _unpack(wo_v[:, _tile(t)]))
        xr = x_v[pl.ds(al(b * T + r0, 16), M), _tile(t)].astype(_F32)
        ob_v[c % 2, :, _tile(t)] = (xr + out).astype(ob_v.dtype)
        return out

    def out_copy(c):
        return pltpu.make_async_copy(ob_v.at[c % 2], o_hbm.at[pl.ds(al(c * M, 16), M)], out_sems.at[c % 2])

    def x_rows(r0, rows):
        return x_v.at[pl.ds(al(r0, 16), rows)]

    def norm_rows(src_ref, dst_ref, r, gate=_no_gate):
        xs = gate(src_ref[r:r + 16, :].astype(_F32))
        dst_ref[r // 2:r // 2 + 8, :] = _pack(_layernorm(xs))

    def g_norm(r, gate=_no_gate):
        g = gate(jnp.concatenate([gn_v[t, r:r + 16, :] for t in range(nl)], axis=1))
        g = _layernorm(g)
        for t in range(nl):
            gn_v[t, r:r + 16, :] = g[:, _tile(t)]

    def max_rows(j, r, first, last, gate=_no_gate):
        cm = gate(s_v[j, r:r + 16, _tile(0)])
        if not first:
            cm = jnp.maximum(cm, mx_v[r:r + 16, :])
        for t in range(1, nc):
            cm = jnp.maximum(cm, s_v[j, r:r + 16, _tile(t)])
        if last:
            m_v[r:r + 16, :] = jnp.broadcast_to(jnp.max(cm, axis=-1, keepdims=True), cm.shape)
        else:
            mx_v[r:r + 16, :] = cm

    def exp_rows(j, buf, r, first, tiles=nc, gate=_no_gate):
        m = gate(m_v[r:r + 16, :])
        l = None if first else l_v[r:r + 16, :]
        p = jnp.exp2(s_v[j, r:r + 16, :tiles * _LANES] - jnp.tile(m, (1, tiles)))
        for t in range(tiles):
            l = p[:, _tile(t)] if l is None else l + p[:, _tile(t)]
        p_v[(buf * M + r) // 2:(buf * M + r) // 2 + 8, :tiles * _LANES] = _pack(p)
        l_v[r:r + 16, :] = l

    def scale_rows(r, tail, gate=_no_gate):
        l = gate(l_v[r:r + 16, :])
        if tail:
            l = l + lt_v[r:r + 16, :]
        inv = 1.0 / jnp.sum(l, axis=-1, keepdims=True)
        for t in range(nl):
            z_v[r // 2:r // 2 + 8, _tile(nl + t)] = _pack(acc_v[t, r:r + 16, :] * inv)

    def conv_piece(t, r, rows, gate=_no_gate):
        off = _HALO - K // 2
        conv = None
        for sh in range(8):
            taps = [i for i in range(K) if (off + i) % 8 == sh]
            span = (off + taps[-1]) // 8 * 8
            slab = cv_v[t, pl.ds(r + sh, rows + span), :]
            for i in taps:
                a = (off + i) // 8 * 8
                term = slab[a:a + rows] * jnp.tile(gate(dwf_v[t, i]), (rows // 8, 1))
                conv = term if conv is None else conv + term
        return _pack(u_v[t, pl.ds(r, rows), :] * conv)

    def conv_to_z(t, r, rows, gate=_no_gate):
        z_v[r // 2:(r + rows) // 2, _tile(t)] = conv_piece(t, r, rows, gate)

    def window_head(n):
        _, r0 = blk_pos(n)
        for t in range(nl):
            cv_v[t, _HALO + M:2 * _HALO + M, :] = jnp.where(r0 > 0, gn_v[t, :_HALO, :], 0.0)

    def advance_window(n, t):
        _, r0 = blk_pos(n)
        if isinstance(n, int):
            cv_v[t, :_HALO, :] = jnp.zeros((_HALO, _LANES), _F32)
        else:
            cv_v[t, :_HALO, :] = jnp.where(r0 > 0, cv_v[t, M:M + _HALO, :], 0.0)
        cv_v[t, _HALO:_HALO + M, :] = gn_v[t]

    class Plan:
        def __init__(self):
            self.order, self.slots = [], {}

        def add(self, name, fns):
            self.slots[name] = list(range(len(self.order), len(self.order) + len(fns)))
            self.order += [(f, []) for f in fns]

        def insert(self, fns, name):
            for f, slot in zip(fns, self.slots[name], strict=True):
                self.order[slot][1].append((slot, -1.0, lambda gate, f=f: f()))

        def spread(self, fns, *names, skip=0, defer=False):
            slots = [i for name in names for i in self.slots[name]]
            for k, f in enumerate(fns):
                pos = k * (len(slots) - skip) / len(fns)
                slot = slots[int(pos)]
                self.order[slots[-1] if defer else slot][1].append((slot, pos - int(pos), f))

        def run(self):
            keep = one_v[...] != 0
            res = []
            for f, fillers in self.order:
                res.append(f())
                for slot, frac, filler in sorted(fillers, key=lambda e: e[:2]):
                    r = int(max(frac, 0.0) * (res[slot].shape[0] // 8)) * 8

                    def gate(x, g=res[slot][r:r + 8, :_LANES]):
                        reps = (x.shape[0] // 8, x.shape[1] // _LANES)
                        return jnp.where(jnp.tile(keep, reps), x, jnp.tile(g, reps))

                    filler(gate=gate)

    P = functools.partial
    rows16 = range(0, M, 16)
    conv_rows = [(r, min(_CONV_ROWS, M - r)) for r in range(0, M, _CONV_ROWS)]
    conv_rows_last = [(r, min(_CONV_ROWS_LAST, M - r)) for r in range(0, M, _CONV_ROWS_LAST)]

    def first_step():
        def cp(src, dst, i):
            return pltpu.make_async_copy(src, dst, sems.at[i])

        def cx(j):
            r = al(j * C, C)
            return cp(x_hbm.at[pl.ds(r, C), :], x_v.at[pl.ds(r, C), :], 10 + j)

        c_wq, c_wk, c_wup = cp(wq_hbm, wq_v, 0), cp(wk_hbm, wk_v, 1), cp(wup_hbm, wupin_v, 2)
        c_w = [cp(wv_hbm, wv_v, 3), cp(wao_hbm, wao_v, 4), cp(wdn_hbm, wdn_v, 5), cp(wm_hbm, wm_v, 6)]
        c_dw = cp(dw_hbm, dw_v, 8)
        c_rest = cp(x_hbm.at[pl.ds(TP, B * T - TP), :], x_v.at[pl.ds(TP, B * T - TP), :], 9)
        for c in [c_wq, c_wk, cx(0), c_wup] + [cx(j) for j in range(1, nchunk)] + c_w + [c_dw, c_rest]:
            c.start()

        one_v[...] = jnp.ones(one_v.shape, jnp.int32)
        mx_v[...] = jnp.full(mx_v.shape, -jnp.inf, _F32)

        def a_tile(t):
            a = _dot_nt(wq_v[...], wk_v[_tile(t), :])
            a_v[:, _tile(t)] = _pack(a * (float(D) ** -0.5 * math.log2(math.e)))
            return a

        c_wq.wait()
        c_wk.wait()
        cx(0).wait()
        plan = Plan()
        plan.add("a", [P(a_tile, t) for t in range(nl)])
        plan.spread([P(norm_rows, x_v, xa_v, r) for r in range(0, C, 16)], "a", skip=2)
        plan.run()
        select_rows(0)
        c_wup.wait()
        cx(1).wait()
        wup_v[...] = pltpu.bitcast(wupin_v[...], _U32)
        plan = Plan()
        plan.add("g", [P(g_tile, 0, t) for t in range(nl)])
        plan.add("q", [P(q_tile, 0, t) for t in range(nl)])
        plan.add("u", [P(u_tile, 0, t) for t in range(nl)])
        plan.spread([P(g_norm, r) for r in rows16], "q")
        plan.spread([P(norm_rows, x_v, xa_v, C + r) for r in range(0, C, 16)], "g", "u", skip=1)
        plan.run()
        for t in range(nl):
            advance_window(0, t)

        def qk_body(it, carry):
            for jj in range(_UNROLL):
                j = it * _UNROLL + jj
                if jj + 2 < _UNROLL:
                    cx(j + 2).wait()
                else:
                    pl.when(j + 2 < nchunk)(lambda: cx(j + 2).wait())
            plan = Plan()
            for jj in range(_UNROLL):
                j = it * _UNROLL + jj
                plan.add(jj, [P(qk_tile, 0, j, t, jj == _UNROLL - 1, True) for t in range(nc)])
                nxt = jnp.minimum(j + 2, nchunk - 1)
                src, dst = x_rows(nxt * C, C), xa_v.at[pl.ds(al(nxt * (C // 2), 8), C // 2)]
                plan.spread([P(norm_rows, src, dst, r) for r in range(0, C, 16)], jj, skip=_QK_SKIP, defer=True)
            plan.run()
            return carry

        jax.lax.fori_loop(0, nchunk // _UNROLL, qk_body, 0)
        for c in c_w + [c_dw, c_rest]:
            c.wait()

        def fold_tile(lhs, rhs_rows, dst, t):
            w = _dot(lhs[...], wm_v[rhs_rows, _tile(t)] if rhs_rows is not None else wao_v[:, _tile(t)])
            dst(t, w)
            return w

        def to_wvo(t, w):
            wvo_v[:, _tile(t)] = w.astype(_BF16)

        def to_wo(half, t, w):
            wo_v[half * D // 2:(half + 1) * D // 2, _tile(t)] = _pack(w)

        def taps(t, gate):
            wt = dw_v[:, _tile(t)].astype(_F32)
            for i in range(K):
                dwf_v[t, i] = jnp.broadcast_to(wt[i:i + 1], (8, _LANES))

        def finish_max(r, gate):
            cm = gate(mx_v[r:r + 16, :])
            m_v[r:r + 16, :] = jnp.broadcast_to(jnp.max(cm, axis=-1, keepdims=True), cm.shape)

        plan = Plan()
        plan.add("vo", [P(fold_tile, wv_v, None, to_wvo, t) for t in range(nl)])
        plan.add("dm", [P(fold_tile, wdn_v, slice(D, 2 * D), P(to_wo, 0), t) for t in range(nl)])
        plan.add("vom", [P(fold_tile, wvo_v, slice(0, D), P(to_wo, 1), t) for t in range(nl)])
        plan.spread([P(finish_max, r) for r in rows16], "vo")
        plan.spread([P(taps, t) for t in range(nl)], "dm")
        plan.run()
        for b in range(B):
            xa_v[xa_rows(b * TP + T, TP - T), :] = jnp.zeros(((TP - T) // 2, D), _U32)
        select_rows(1)

    def middle_step(n, carry):
        c = n - 1
        pl.when(c >= 2)(lambda: out_copy(c - 2).wait())
        last = nchunk - 1
        cuts = [8 * x for x in _CUTS]
        plan = Plan()
        plan.add("q", [P(q_tile, n, t) for t in range(nl)])
        plan.add(("pv", 0), [P(pv_tile, c, 0, t, 0, True) for t in range(nl)])
        plan.add("g", [P(g_tile, n, t) for t in range(nl)])
        for j in range(last):
            plan.add(("qk", j), [P(qk_tile, n, j, t, False, False) for t in range(nc)])
            keys = C - _LANES if (j + 1 == last and _E2) else C
            plan.add(("pv", j + 1), [P(pv_tile, c, j + 1, t, (j + 1) % 2, False, keys,
                                       (cuts[j], cuts[j + 1]) if _E2 else None) for t in range(nl)])
        if _E1:
            plan.add(("qk", last), [P(qk_tile, n, last, t, False, False) for t in range(nc - 1)])
            plan.insert([P(qk_tail, n, i) for i in range(pl.cdiv(M, _LANES))], ("pv", last))
        else:
            plan.add(("qk", last), [P(qk_tile, n, last, t, True, False) for t in range(nc)])
        plan.add("u", [P(u_tile, n, t) for t in range(nl)])
        plan.add("out", [P(out_tile, c, t) for t in range(nl)])

        for j in range(last):
            tiles = nc - 1 if (j + 1 == last and _E2) else nc
            plan.spread([P(exp_rows, j + 1, (j + 1) % 2, r, False, tiles) for r in rows16], ("pv", j), ("qk", j))
            plan.spread([P(max_rows, j, r, j == 0, False) for r in rows16], ("pv", j + 1))
        plan.spread([P(g_norm, r) for r in rows16[:1]] + [lambda gate: window_head(n)]
                    + [P(g_norm, r) for r in rows16[1:]], ("qk", 0), ("pv", 1))
        plan.spread([P(conv_to_z, t, r, rows) for r, rows in conv_rows for t in range(nl)],
                    *[(name, j + d) for j in range(_CONV_FROM, _CONV_TO) for name, d in (("qk", 0), ("pv", 1))])
        plan.spread([P(scale_rows, r, _E2) for r in rows16], ("qk", last))
        if _E2:
            tail_values(c)
            for j in range(last):
                names = (("pv", j), ("qk", j)) if j else ("q", ("pv", 0), "g", ("qk", 0))
                plan.spread([P(pv_tail, r) for r in range(cuts[j], cuts[j + 1], 8)], *names, skip=_TSKIP)
        plan.spread([P(max_rows, last, r, False, True) for r in rows16], "out", skip=1)
        def piece(i):
            return jnp.clip(i * (NR // 2), 0, (T - NR) // 2)

        copy_rows(TP // 2 + piece(c - 1), NR // 2)
        src = x_rows(T + 2 * piece(c), NR)
        plan.spread([P(norm_rows, src, st_v, r) for r in range(0, NR, 16)], *_NORM_AT)

        for r in rows16:
            exp_rows(0, 0, r, True)
        plan.run()
        select_rows(jnp.minimum(n + 1, total - 1))
        for t in range(nl):
            advance_window(n, t)
        out_copy(c).start()
        return carry

    def last_step():
        c = total - 1
        out_copy(c - 2).wait()
        nit = nchunk // _UNROLL
        for t in range(nl):
            cv_v[t, _HALO + M:2 * _HALO + M, :] = jnp.zeros((_HALO, _LANES), _F32)
        l_v[...] = jnp.zeros(l_v.shape, _F32)
        acc_v[...] = jnp.zeros(acc_v.shape, _F32)

        def conv_to_st(t, r, rows, gate):
            gn_v[t, r // 2:(r + rows) // 2, :] = pltpu.bitcast(conv_piece(t, r, rows, gate), _F32)

        def pv_body(it, carry):
            plan = Plan()
            for jj in range(_UNROLL):
                j = it * _UNROLL + jj
                plan.add(jj, [P(pv_tile, c, j, t, jj % 2, False) for t in range(nl)])
                if jj + 1 < _UNROLL:
                    plan.spread([P(exp_rows, j + 1, (jj + 1) % 2, r, False) for r in rows16], jj, skip=1)
            plan.spread([P(conv_to_st, it * (nl // nit) + tt, r, rows)
                         for tt in range(nl // nit) for r, rows in conv_rows_last], *range(_UNROLL), skip=1)
            for r in rows16:
                exp_rows(it * _UNROLL, 0, r, False)
            plan.run()
            return carry

        jax.lax.fori_loop(0, nit, pv_body, 0)
        for t in range(nl):
            z_v[:, _tile(t)] = pltpu.bitcast(gn_v[t, :M // 2, :], _U32)
        for r in rows16:
            scale_rows(r, False)
        for t in range(nl):
            out_tile(c, t)
        out_copy(c).start()
        out_copy(c - 1).wait()
        out_copy(c).wait()

    with jax.named_scope("first"):
        first_step()
    with jax.named_scope("main"):
        jax.lax.fori_loop(1, total, middle_step, 0)
    with jax.named_scope("last"):
        last_step()


@jax.jit
def pallas_standalone__conformer_family_branchformer__speech_kernel(
    x: jax.Array,
    w_q: jax.Array,
    w_k: jax.Array,
    w_v: jax.Array,
    w_ao: jax.Array,
    w_up: jax.Array,
    dw: jax.Array,
    w_dn: jax.Array,
    w_merge: jax.Array,
):
    B, T, D = x.shape
    K = dw.shape[0]
    M, C = _BLK, _CHUNK
    assert T % M == 0 and D % _LANES == 0 and K // 2 <= _HALO and B == 2
    nblk = T // M
    total = B * nblk
    TP = pl.cdiv(T, C) * C
    nl = D // _LANES
    NR = _norm_rows_per_step(T)

    vmem = pltpu.VMEM
    return pl.pallas_call(
        functools.partial(_kernel, B=B, T=T, D=D, K=K),
        in_specs=[pl.BlockSpec(memory_space=pl.ANY)] * 9,
        out_specs=pl.BlockSpec(memory_space=pl.ANY),
        out_shape=jax.ShapeDtypeStruct((B * T, D), x.dtype),
        scratch_shapes=[
            vmem((B * T, D), x.dtype),
            vmem((D, D), w_q.dtype), vmem((D, D), w_k.dtype), vmem((D, 2 * D), w_up.dtype),
            vmem((K, D), dw.dtype),
            vmem((D, D), w_v.dtype), vmem((D, D), w_ao.dtype), vmem((D, D), w_dn.dtype),
            vmem((2 * D, D), w_merge.dtype),
            vmem((D, D), _BF16),
            vmem((NR // 2, D), _U32),
            vmem((M // 2, D), _U32),
            vmem((D // 2, D), _U32),
            vmem((D // 2, 2 * D), _U32),
            vmem((D, D), _U32),
            vmem((nl, K, 8, _LANES), _F32),
            vmem((B * TP // 2, D), _U32),
            vmem((nl, M + 2 * _HALO, _LANES), _F32),
            vmem((nl, M, _LANES), _F32),
            vmem((nl, M, _LANES), _F32),
            vmem((TP // C, M, C), _F32),
            vmem((M, _LANES), _F32),
            vmem((M, _LANES), _F32),
            vmem((M, _LANES), _F32),
            vmem((nl, M, _LANES), _F32),
            vmem((M // 2, D), _U32),
            vmem((M, C), _U32),
            vmem((M // 2, 2 * D), _U32),
            vmem((8, _LANES), jnp.int32),
            vmem((T % _LANES, nl, 8, _LANES), _F32),
            vmem((M, _LANES), _F32),
            vmem((nl, M, _LANES), _F32),
            vmem((2, M, D), x.dtype),
            pltpu.SemaphoreType.DMA((10 + TP // C,)),
            pltpu.SemaphoreType.DMA((2,)),
        ],
        compiler_params=pltpu.CompilerParams(
            vmem_limit_bytes=110 * 2**20,
            flags=_FLAGS,
        ),
    )(x.reshape(B * T, D), w_q, w_k, w_v, w_ao, w_up, dw, w_dn, w_merge).reshape(B, T, D)
```

```python
import functools
import math

import jax
import jax.numpy as jnp
import jax.experimental.pallas as pl
import jax.experimental.pallas.tpu as pltpu

_EPS = 1e-5
_LANES = 128
_BLK = 400
_CHUNK = 512
_HALO = 16
_GELU_C = math.sqrt(2.0 / math.pi)
_UNROLL = 4
_CONV_ROWS = 16
_CONV_ROWS_LAST = 16
_QK_SKIP = 2
_AHEAD = 1
_E1 = True
_E2 = False
_CUTS = (0, 14, 20, 26, 32, 38, 44, 50)
_TSKIP = 0
_LAG = 2
_TAIL_AT = ("q", ("pv", 0), "g", ("qk", 0), ("pv", 1), ("qk", 1), ("pv", 2), ("qk", 2), ("pv", 3), ("qk", 3), ("pv", 4), ("qk", 4), ("pv", 5), ("qk", 5))
_CONV_FROM = 1
_CONV_TO = 6
_FLAGS = None
_NORM_AT = (("pv", 0), "g")

_F32 = jnp.float32
_BF16 = jnp.bfloat16
_U32 = jnp.uint32


def _dot(a, b):
    return jax.lax.dot_general(a, b, (((1,), (0,)), ((), ())), preferred_element_type=_F32)


def _dot_nt(a, b):
    return jax.lax.dot_general(a, b, (((1,), (1,)), ((), ())), preferred_element_type=_F32)


def _pack(x):
    return pltpu.bitcast(x.astype(_BF16), _U32)


def _unpack(w):
    return pltpu.bitcast(w, _BF16)


def _layernorm(x):
    m = jnp.mean(x, axis=-1, keepdims=True)
    xc = x - m
    v = jnp.mean(xc * xc, axis=-1, keepdims=True)
    return xc * jax.lax.rsqrt(v + _EPS)


def _gelu(x):
    inner = x * (_GELU_C + (_GELU_C * 0.044715) * (x * x))
    hx = 0.5 * x
    return hx + hx * jnp.tanh(inner)


def _tile(t):
    return slice(t * _LANES, (t + 1) * _LANES)


def _no_gate(x):
    return x


def _norm_rows_per_step(T):
    return pl.cdiv(T, 16 * (T // _BLK - 1)) * 16


def _kernel(x_hbm, wq_hbm, wk_hbm, wv_hbm, wao_hbm, wup_hbm, dw_hbm, wdn_hbm, wm_hbm,
            o_hbm,
            x_v, wq_v, wk_v, wupin_v, dw_v, wv_v, wao_v, wdn_v, wm_v, wvo_v, st_v, xq_v,
            a_v, wup_v, wo_v, dwf_v, xa_v, cv_v, gn_v, u_v, s_v, m_v, mx_v, l_v, acc_v, q_v, p_v, z_v,
            one_v, vt_v, lt_v, acct_v, ob_v, sems, out_sems,
            *, B, T, D, K):
    M, C = _BLK, _CHUNK
    nblk = T // M
    total = B * nblk
    TP = pl.cdiv(T, C) * C
    nchunk = TP // C
    nl = D // _LANES
    nc = C // _LANES
    TAIL = T % _LANES
    NR = _norm_rows_per_step(T)

    def blk_pos(n):
        if isinstance(n, int):
            return n // nblk, (n % nblk) * M
        b = n // nblk
        return b, pl.multiple_of((n - b * nblk) * M, 16)

    def al(v, mult):
        return v if isinstance(v, int) else pl.multiple_of(v, mult)

    def xa_rows(r, rows):
        return pl.ds(al(r // 2, 8), rows // 2)

    def select_rows(n):
        b, r0 = blk_pos(n)
        xq_v[...] = xa_v[xa_rows(b * TP + r0, M), :]

    def xq():
        return _unpack(xq_v[...])

    def q_tile(n, t):
        q = _dot(xq(), _unpack(a_v[:, _tile(t)]))
        q_v[:, _tile(t)] = _pack(q)
        return q

    def g_tile(n, t):
        h = _dot(xq(), _unpack(wup_v[:, _tile(nl + t)]))
        gn_v[t] = _gelu(h)
        return h

    def u_tile(n, t):
        h = _dot(xq(), _unpack(wup_v[:, _tile(t)]))
        u_v[t] = _gelu(h)
        return h

    def copy_rows(dst0, rows):
        xa_v[pl.ds(al(dst0, 8), rows), :] = st_v[...]

    def qk_tile(n, j, t, mask, track_max):
        b, _ = blk_pos(n)
        k = _unpack(xa_v[xa_rows(b * TP + j * C + t * _LANES, _LANES), :])
        s = _dot_nt(_unpack(q_v[...]), k)
        if mask and t == nc - 1:
            col = jax.lax.broadcasted_iota(jnp.int32, s.shape, 1)
            s = jnp.where(col < T - j * C - t * _LANES, s, -jnp.inf)
        s_v[j, :, _tile(t)] = s
        if track_max:
            mx_v[...] = jnp.maximum(mx_v[...], s)
        return s

    def qk_tail(n, i):
        b, _ = blk_pos(n)
        r, rows = i * _LANES, min(_LANES, M - i * _LANES)
        q = _unpack(q_v[r // 2:(r + rows) // 2, :])
        if rows == _LANES:
            s = _dot_nt(_unpack(xa_v[xa_rows(b * TP + T - TAIL, TAIL), :]), q)
            pad = jnp.full((_LANES - TAIL, _LANES), -jnp.inf, _F32)
            s = jnp.concatenate([s, pad], axis=0).T
        else:
            s = _dot_nt(q, _unpack(xa_v[xa_rows(b * TP + T - TAIL, _LANES), :]))
            col = jax.lax.broadcasted_iota(jnp.int32, s.shape, 1)
            s = jnp.where(col < TAIL, s, -jnp.inf)
        s_v[nchunk - 1, r:r + rows, _tile(nc - 1)] = s
        return s

    def tail_values(c):
        b, _ = blk_pos(c)
        v = _unpack(xa_v[xa_rows(b * TP + T - TAIL, TAIL), :]).astype(_F32)
        for k in range(TAIL):
            for t in range(nl):
                vt_v[k, t] = jnp.broadcast_to(v[k:k + 1, _tile(t)], (8, _LANES))

    def pv_tail(r, gate=_no_gate):
        p = jnp.exp2(s_v[nchunk - 1, r:r + 8, _tile(nc - 1)] - gate(m_v[r:r + 8, :]))
        lt_v[r:r + 8, :] = p
        acc = [None] * nl
        done = []
        keep = one_v[...] != 0
        for k in range(TAIL):
            if k >= _LAG:
                p = jnp.where(keep, p, done[k - _LAG])
            pk = jnp.broadcast_to(p[:, k:k + 1], (8, _LANES))
            for t in range(nl):
                term = pk * vt_v[k, t]
                acc[t] = term if k == 0 else acc[t] + term
            done.append(acc[k % nl])
        for t in range(nl):
            acct_v[t, r:r + 8, :] = acc[t]

    def pv_tile(c, j, t, buf, first, keys=C, tail_rows=None):
        b, _ = blk_pos(c)
        v = _unpack(xa_v[xa_rows(b * TP + j * C, keys), _tile(t)])
        pv = _dot(_unpack(p_v[buf * M // 2:(buf + 1) * M // 2, :keys]), v)
        acc = pv if first else acc_v[t] + pv
        if tail_rows is None:
            acc_v[t] = acc
        else:
            lo, hi = tail_rows
            if lo > 0:
                acc_v[t, :lo, :] = acc[:lo]
            acc_v[t, lo:hi, :] = acc[lo:hi] + acct_v[t, lo:hi, :]
            if hi < M:
                acc_v[t, hi:, :] = acc[hi:]
        return pv

    def out_tile(c, t):
        b, r0 = blk_pos(c)
        out = _dot(_unpack(z_v[...]), _unpack(wo_v[:, _tile(t)]))
        xr = x_v[pl.ds(al(b * T + r0, 16), M), _tile(t)].astype(_F32)
        ob_v[c % 2, :, _tile(t)] = (xr + out).astype(ob_v.dtype)
        return out

    def out_copy(c):
        return pltpu.make_async_copy(ob_v.at[c % 2], o_hbm.at[pl.ds(al(c * M, 16), M)], out_sems.at[c % 2])

    def x_rows(r0, rows):
        return x_v.at[pl.ds(al(r0, 16), rows)]

    def norm_rows(src_ref, dst_ref, r, gate=_no_gate):
        xs = gate(src_ref[r:r + 16, :].astype(_F32))
        dst_ref[r // 2:r // 2 + 8, :] = _pack(_layernorm(xs))

    def g_norm(r, gate=_no_gate):
        g = gate(jnp.concatenate([gn_v[t, r:r + 16, :] for t in range(nl)], axis=1))
        g = _layernorm(g)
        for t in range(nl):
            gn_v[t, r:r + 16, :] = g[:, _tile(t)]

    def max_rows(j, r, first, last, gate=_no_gate):
        cm = gate(s_v[j, r:r + 16, _tile(0)])
        if not first:
            cm = jnp.maximum(cm, mx_v[r:r + 16, :])
        for t in range(1, nc):
            cm = jnp.maximum(cm, s_v[j, r:r + 16, _tile(t)])
        if last:
            m_v[r:r + 16, :] = jnp.broadcast_to(jnp.max(cm, axis=-1, keepdims=True), cm.shape)
        else:
            mx_v[r:r + 16, :] = cm

    def exp_rows(j, buf, r, first, tiles=nc, gate=_no_gate):
        m = gate(m_v[r:r + 16, :])
        l = None if first else l_v[r:r + 16, :]
        p = jnp.exp2(s_v[j, r:r + 16, :tiles * _LANES] - jnp.tile(m, (1, tiles)))
        for t in range(tiles):
            l = p[:, _tile(t)] if l is None else l + p[:, _tile(t)]
        p_v[(buf * M + r) // 2:(buf * M + r) // 2 + 8, :tiles * _LANES] = _pack(p)
        l_v[r:r + 16, :] = l

    def scale_rows(r, tail, gate=_no_gate):
        l = gate(l_v[r:r + 16, :])
        if tail:
            l = l + lt_v[r:r + 16, :]
        inv = 1.0 / jnp.sum(l, axis=-1, keepdims=True)
        for t in range(nl):
            z_v[r // 2:r // 2 + 8, _tile(nl + t)] = _pack(acc_v[t, r:r + 16, :] * inv)

    def conv_piece(t, r, rows, gate=_no_gate):
        off = _HALO - K // 2
        conv = None
        for sh in range(8):
            taps = [i for i in range(K) if (off + i) % 8 == sh]
            span = (off + taps[-1]) // 8 * 8
            slab = cv_v[t, pl.ds(r + sh, rows + span), :]
            for i in taps:
                a = (off + i) // 8 * 8
                term = slab[a:a + rows] * jnp.tile(gate(dwf_v[t, i]), (rows // 8, 1))
                conv = term if conv is None else conv + term
        return _pack(u_v[t, pl.ds(r, rows), :] * conv)

    def conv_to_z(t, r, rows, gate=_no_gate):
        z_v[r // 2:(r + rows) // 2, _tile(t)] = conv_piece(t, r, rows, gate)

    def window_head(n):
        _, r0 = blk_pos(n)
        for t in range(nl):
            cv_v[t, _HALO + M:2 * _HALO + M, :] = jnp.where(r0 > 0, gn_v[t, :_HALO, :], 0.0)

    def advance_window(n, t):
        _, r0 = blk_pos(n)
        if isinstance(n, int):
            cv_v[t, :_HALO, :] = jnp.zeros((_HALO, _LANES), _F32)
        else:
            cv_v[t, :_HALO, :] = jnp.where(r0 > 0, cv_v[t, M:M + _HALO, :], 0.0)
        cv_v[t, _HALO:_HALO + M, :] = gn_v[t]

    class Plan:
        def __init__(self):
            self.order, self.slots = [], {}

        def add(self, name, fns):
            self.slots[name] = list(range(len(self.order), len(self.order) + len(fns)))
            self.order += [(f, []) for f in fns]

        def insert(self, fns, name):
            for f, slot in zip(fns, self.slots[name], strict=True):
                self.order[slot][1].append((slot, -1.0, lambda gate, f=f: f()))

        def spread(self, fns, *names, skip=0, defer=False):
            slots = [i for name in names for i in self.slots[name]]
            for k, f in enumerate(fns):
                pos = k * (len(slots) - skip) / len(fns)
                slot = slots[int(pos)]
                self.order[slots[-1] if defer else slot][1].append((slot, pos - int(pos), f))

        def run(self):
            keep = one_v[...] != 0
            res = []
            for f, fillers in self.order:
                res.append(f())
                for slot, frac, filler in sorted(fillers, key=lambda e: e[:2]):
                    r = int(max(frac, 0.0) * (res[slot].shape[0] // 8)) * 8

                    def gate(x, g=res[slot][r:r + 8, :_LANES]):
                        reps = (x.shape[0] // 8, x.shape[1] // _LANES)
                        return jnp.where(jnp.tile(keep, reps), x, jnp.tile(g, reps))

                    filler(gate=gate)

    P = functools.partial
    rows16 = range(0, M, 16)
    conv_rows = [(r, min(_CONV_ROWS, M - r)) for r in range(0, M, _CONV_ROWS)]
    conv_rows_last = [(r, min(_CONV_ROWS_LAST, M - r)) for r in range(0, M, _CONV_ROWS_LAST)]

    def first_step():
        def cp(src, dst, i):
            return pltpu.make_async_copy(src, dst, sems.at[i])

        def cx(j):
            r = al(j * C, C)
            return cp(x_hbm.at[pl.ds(r, C), :], x_v.at[pl.ds(r, C), :], 10 + j)

        halves = [pl.ds(h * D // 2, D // 2) for h in range(2)]
        c_wq = [cp(wq_hbm.at[h], wq_v.at[h], i) for h, i in zip(halves, (0, 7))]
        c_wk, c_wup = cp(wk_hbm, wk_v, 1), cp(wup_hbm, wupin_v, 2)
        c_w = [cp(wv_hbm, wv_v, 3), cp(wao_hbm, wao_v, 4), cp(wdn_hbm, wdn_v, 5), cp(wm_hbm, wm_v, 6)]
        c_dw = cp(dw_hbm, dw_v, 8)
        c_rest = cp(x_hbm.at[pl.ds(TP, B * T - TP), :], x_v.at[pl.ds(TP, B * T - TP), :], 9)
        for c in [c_wk] + c_wq + [cx(0), c_wup] + [cx(j) for j in range(1, nchunk)] + c_w + [c_dw, c_rest]:
            c.start()

        one_v[...] = jnp.ones(one_v.shape, jnp.int32)
        mx_v[...] = jnp.full(mx_v.shape, -jnp.inf, _F32)

        def a_tile(h, t):
            a = _dot_nt(wq_v[halves[h]], wk_v[_tile(t), :])
            a_v[h * D // 4:(h + 1) * D // 4, _tile(t)] = _pack(a * (float(D) ** -0.5 * math.log2(math.e)))
            return a

        c_wk.wait()
        c_wq[0].wait()
        for t in range(nl):
            a_tile(0, t)
        c_wq[1].wait()
        cx(0).wait()
        plan = Plan()
        plan.add("a", [P(a_tile, 1, t) for t in range(nl)])
        plan.spread([P(norm_rows, x_v, xa_v, r) for r in range(0, C, 16)], "a", skip=2)
        plan.run()
        select_rows(0)
        for t in range(nl):
            q_tile(0, t)
        c_wup.wait()
        if _AHEAD == 2:
            cx(1).wait()
        wup_v[...] = pltpu.bitcast(wupin_v[...], _U32)
        plan = Plan()
        plan.add("g", [P(g_tile, 0, t) for t in range(nl)])
        plan.add("u", [P(u_tile, 0, t) for t in range(nl)])
        if _AHEAD == 2:
            plan.spread([P(norm_rows, x_v, xa_v, C + r) for r in range(0, C, 16)], "g")
        plan.spread([P(g_norm, r) for r in rows16], "u", skip=1)
        plan.run()
        for t in range(nl):
            advance_window(0, t)

        def qk_body(it, carry):
            for jj in range(_UNROLL):
                j = it * _UNROLL + jj
                if jj + _AHEAD < _UNROLL:
                    cx(j + _AHEAD).wait()
                else:
                    pl.when(j + _AHEAD < nchunk)(lambda: cx(j + _AHEAD).wait())
            plan = Plan()
            for jj in range(_UNROLL):
                j = it * _UNROLL + jj
                plan.add(jj, [P(qk_tile, 0, j, t, jj == _UNROLL - 1, True) for t in range(nc)])
                nxt = jnp.minimum(j + _AHEAD, nchunk - 1)
                src, dst = x_rows(nxt * C, C), xa_v.at[pl.ds(al(nxt * (C // 2), 8), C // 2)]
                plan.spread([P(norm_rows, src, dst, r) for r in range(0, C, 16)], jj, skip=_QK_SKIP, defer=True)
            plan.run()
            return carry

        jax.lax.fori_loop(0, nchunk // _UNROLL, qk_body, 0)
        for c in c_w + [c_dw]:
            c.wait()

        def fold_tile(lhs, rhs_rows, dst, t):
            w = _dot(lhs[...], wm_v[rhs_rows, _tile(t)] if rhs_rows is not None else wao_v[:, _tile(t)])
            dst(t, w)
            return w

        def to_wvo(t, w):
            wvo_v[:, _tile(t)] = w.astype(_BF16)

        def to_wo(half, t, w):
            wo_v[half * D // 2:(half + 1) * D // 2, _tile(t)] = _pack(w)

        def taps(t, gate):
            wt = dw_v[:, _tile(t)].astype(_F32)
            for i in range(K):
                dwf_v[t, i] = jnp.broadcast_to(wt[i:i + 1], (8, _LANES))

        def finish_max(r, gate):
            cm = gate(mx_v[r:r + 16, :])
            m_v[r:r + 16, :] = jnp.broadcast_to(jnp.max(cm, axis=-1, keepdims=True), cm.shape)

        plan = Plan()
        plan.add("vo", [P(fold_tile, wv_v, None, to_wvo, t) for t in range(nl)])
        plan.add("dm", [P(fold_tile, wdn_v, slice(D, 2 * D), P(to_wo, 0), t) for t in range(nl)])
        plan.add("vom", [P(fold_tile, wvo_v, slice(0, D), P(to_wo, 1), t) for t in range(nl)])
        plan.spread([P(finish_max, r) for r in rows16], "vo")
        plan.spread([P(taps, t) for t in range(nl)], "dm")
        plan.run()
        for b in range(B):
            xa_v[xa_rows(b * TP + T, TP - T), :] = jnp.zeros(((TP - T) // 2, D), _U32)
        select_rows(1)
        c_rest.wait()

    def middle_step(n, carry):
        c = n - 1
        pl.when(c >= 2)(lambda: out_copy(c - 2).wait())
        last = nchunk - 1
        cuts = [8 * x for x in _CUTS]
        plan = Plan()
        plan.add("q", [P(q_tile, n, t) for t in range(nl)])
        plan.add(("pv", 0), [P(pv_tile, c, 0, t, 0, True) for t in range(nl)])
        plan.add("g", [P(g_tile, n, t) for t in range(nl)])
        for j in range(last):
            plan.add(("qk", j), [P(qk_tile, n, j, t, False, False) for t in range(nc)])
            keys = C - _LANES if (j + 1 == last and _E2) else C
            plan.add(("pv", j + 1), [P(pv_tile, c, j + 1, t, (j + 1) % 2, False, keys,
                                       (cuts[j], cuts[j + 1]) if _E2 else None) for t in range(nl)])
        if _E1:
            plan.add(("qk", last), [P(qk_tile, n, last, t, False, False) for t in range(nc - 1)])
            plan.insert([P(qk_tail, n, i) for i in range(pl.cdiv(M, _LANES))], ("pv", last))
        else:
            plan.add(("qk", last), [P(qk_tile, n, last, t, True, False) for t in range(nc)])
        plan.add("u", [P(u_tile, n, t) for t in range(nl)])
        plan.add("out", [P(out_tile, c, t) for t in range(nl)])

        for j in range(last):
            tiles = nc - 1 if (j + 1 == last and _E2) else nc
            plan.spread([P(exp_rows, j + 1, (j + 1) % 2, r, False, tiles) for r in rows16], ("pv", j), ("qk", j))
            plan.spread([P(max_rows, j, r, j == 0, False) for r in rows16], ("pv", j + 1))
        plan.spread([P(g_norm, r) for r in rows16[:1]] + [lambda gate: window_head(n)]
                    + [P(g_norm, r) for r in rows16[1:]], ("qk", 0), ("pv", 1))
        plan.spread([P(conv_to_z, t, r, rows) for r, rows in conv_rows for t in range(nl)],
                    *[(name, j + d) for j in range(_CONV_FROM, _CONV_TO) for name, d in (("qk", 0), ("pv", 1))])
        plan.spread([P(scale_rows, r, _E2) for r in rows16], ("qk", last))
        if _E2:
            tail_values(c)
            for j in range(last):
                names = (("pv", j), ("qk", j)) if j else ("q", ("pv", 0), "g", ("qk", 0))
                plan.spread([P(pv_tail, r) for r in range(cuts[j], cuts[j + 1], 8)], *names, skip=_TSKIP)
        plan.spread([P(max_rows, last, r, False, True) for r in rows16], "out", skip=1)
        def piece(i):
            return jnp.clip(i * (NR // 2), 0, (T - NR) // 2)

        copy_rows(TP // 2 + piece(c - 1), NR // 2)
        src = x_rows(T + 2 * piece(c), NR)
        plan.spread([P(norm_rows, src, st_v, r) for r in range(0, NR, 16)], *_NORM_AT)

        for r in rows16:
            exp_rows(0, 0, r, True)
        plan.run()
        select_rows(jnp.minimum(n + 1, total - 1))
        for t in range(nl):
            advance_window(n, t)
        out_copy(c).start()
        return carry

    def last_step():
        c = total - 1
        out_copy(c - 2).wait()
        nit = nchunk // _UNROLL
        for t in range(nl):
            cv_v[t, _HALO + M:2 * _HALO + M, :] = jnp.zeros((_HALO, _LANES), _F32)
        l_v[...] = jnp.zeros(l_v.shape, _F32)
        acc_v[...] = jnp.zeros(acc_v.shape, _F32)

        def conv_to_st(t, r, rows, gate):
            gn_v[t, r // 2:(r + rows) // 2, :] = pltpu.bitcast(conv_piece(t, r, rows, gate), _F32)

        def pv_body(it, carry):
            plan = Plan()
            for jj in range(_UNROLL):
                j = it * _UNROLL + jj
                plan.add(jj, [P(pv_tile, c, j, t, jj % 2, False) for t in range(nl)])
                if jj + 1 < _UNROLL:
                    plan.spread([P(exp_rows, j + 1, (jj + 1) % 2, r, False) for r in rows16], jj, skip=1)
            plan.spread([P(conv_to_st, it * (nl // nit) + tt, r, rows)
                         for tt in range(nl // nit) for r, rows in conv_rows_last], *range(_UNROLL), skip=1)
            for r in rows16:
                exp_rows(it * _UNROLL, 0, r, False)
            plan.run()
            return carry

        jax.lax.fori_loop(0, nit, pv_body, 0)
        for t in range(nl):
            z_v[:, _tile(t)] = pltpu.bitcast(gn_v[t, :M // 2, :], _U32)
        for r in rows16:
            scale_rows(r, False)
        final = [pltpu.make_async_copy(ob_v.at[c % 2, :, _tile(t)], o_hbm.at[pl.ds(c * M, M), _tile(t)], sems.at[t])
                 for t in range(nl)]
        for t in range(nl):
            out_tile(c, t)
            final[t].start()
        out_copy(c - 1).wait()
        for cp in final:
            cp.wait()

    with jax.named_scope("first"):
        first_step()
    with jax.named_scope("main"):
        jax.lax.fori_loop(1, total, middle_step, 0)
    with jax.named_scope("last"):
        last_step()


@jax.jit
def pallas_standalone__conformer_family_branchformer__speech_kernel(
    x: jax.Array,
    w_q: jax.Array,
    w_k: jax.Array,
    w_v: jax.Array,
    w_ao: jax.Array,
    w_up: jax.Array,
    dw: jax.Array,
    w_dn: jax.Array,
    w_merge: jax.Array,
):
    B, T, D = x.shape
    K = dw.shape[0]
    M, C = _BLK, _CHUNK
    assert T % M == 0 and D % _LANES == 0 and K // 2 <= _HALO and B == 2
    nblk = T // M
    total = B * nblk
    TP = pl.cdiv(T, C) * C
    nl = D // _LANES
    NR = _norm_rows_per_step(T)

    vmem = pltpu.VMEM
    return pl.pallas_call(
        functools.partial(_kernel, B=B, T=T, D=D, K=K),
        in_specs=[pl.BlockSpec(memory_space=pl.ANY)] * 9,
        out_specs=pl.BlockSpec(memory_space=pl.ANY),
        out_shape=jax.ShapeDtypeStruct((B * T, D), x.dtype),
        scratch_shapes=[
            vmem((B * T, D), x.dtype),
            vmem((D, D), w_q.dtype), vmem((D, D), w_k.dtype), vmem((D, 2 * D), w_up.dtype),
            vmem((K, D), dw.dtype),
            vmem((D, D), w_v.dtype), vmem((D, D), w_ao.dtype), vmem((D, D), w_dn.dtype),
            vmem((2 * D, D), w_merge.dtype),
            vmem((D, D), _BF16),
            vmem((NR // 2, D), _U32),
            vmem((M // 2, D), _U32),
            vmem((D // 2, D), _U32),
            vmem((D // 2, 2 * D), _U32),
            vmem((D, D), _U32),
            vmem((nl, K, 8, _LANES), _F32),
            vmem((B * TP // 2, D), _U32),
            vmem((nl, M + 2 * _HALO, _LANES), _F32),
            vmem((nl, M, _LANES), _F32),
            vmem((nl, M, _LANES), _F32),
            vmem((TP // C, M, C), _F32),
            vmem((M, _LANES), _F32),
            vmem((M, _LANES), _F32),
            vmem((M, _LANES), _F32),
            vmem((nl, M, _LANES), _F32),
            vmem((M // 2, D), _U32),
            vmem((M, C), _U32),
            vmem((M // 2, 2 * D), _U32),
            vmem((8, _LANES), jnp.int32),
            vmem((T % _LANES, nl, 8, _LANES), _F32),
            vmem((M, _LANES), _F32),
            vmem((nl, M, _LANES), _F32),
            vmem((2, M, D), x.dtype),
            pltpu.SemaphoreType.DMA((10 + TP // C,)),
            pltpu.SemaphoreType.DMA((2,)),
        ],
        compiler_params=pltpu.CompilerParams(
            vmem_limit_bytes=110 * 2**20,
            flags=_FLAGS,
        ),
    )(x.reshape(B * T, D), w_q, w_k, w_v, w_ao, w_up, dw, w_dn, w_merge).reshape(B, T, D)
```

```python
import functools
import math

import jax
import jax.numpy as jnp
import jax.experimental.pallas as pl
import jax.experimental.pallas.tpu as pltpu

_EPS = 1e-5
_LANES = 128
_ROWS = 16
_BLK = 400
_CHUNK = 512
_UNROLL = 4
_HALO = 16
_GELU_C = math.sqrt(2.0 / math.pi)

_F32 = jnp.float32
_BF16 = jnp.bfloat16
_U32 = jnp.uint32


def _dot(a, b):
    return jax.lax.dot_general(a, b, (((1,), (0,)), ((), ())), preferred_element_type=_F32)


def _dot_nt(a, b):
    return jax.lax.dot_general(a, b, (((1,), (1,)), ((), ())), preferred_element_type=_F32)


def _pack(x):
    return pltpu.bitcast(x.astype(_BF16), _U32)


def _unpack(w):
    return pltpu.bitcast(w, _BF16)


def _layernorm(x):
    m = jnp.mean(x, axis=-1, keepdims=True)
    xc = x - m
    v = jnp.mean(xc * xc, axis=-1, keepdims=True)
    return xc * jax.lax.rsqrt(v + _EPS)


def _gelu(x):
    inner = x * (_GELU_C + (_GELU_C * 0.044715) * (x * x))
    hx = 0.5 * x
    return hx + hx * jnp.tanh(inner)


def _tile(t):
    return slice(t * _LANES, (t + 1) * _LANES)


def _no_gate(x):
    return x


def _aligned(v, mult):
    return v if isinstance(v, int) else pl.multiple_of(v, mult)


def _norm_rows_per_step(T):
    return pl.cdiv(T, _ROWS * (T // _BLK - 1)) * _ROWS


class _Plan:
    def __init__(self, ones_ref):
        self.ones_ref = ones_ref
        self.order = []
        self.slots = {}

    def add(self, name, tasks):
        self.slots[name] = list(range(len(self.order), len(self.order) + len(tasks)))
        self.order += [(task, []) for task in tasks]

    def insert(self, tasks, name):
        for task, slot in zip(tasks, self.slots[name], strict=True):
            self.order[slot][1].append((slot, -1.0, lambda gate, task=task: task()))

    def spread(self, pieces, *names, skip=0, defer=False):
        slots = [i for name in names for i in self.slots[name]]
        for k, piece in enumerate(pieces):
            pos = k * (len(slots) - skip) / len(pieces)
            slot = slots[int(pos)]
            self.order[slots[-1] if defer else slot][1].append((slot, pos - int(pos), piece))

    def run(self):
        keep = self.ones_ref[...] != 0
        results = []
        for task, pieces in self.order:
            results.append(task())
            for slot, frac, piece in sorted(pieces, key=lambda e: e[:2]):
                r = int(max(frac, 0.0) * (results[slot].shape[0] // 8)) * 8

                def gate(x, after=results[slot][r:r + 8]):
                    reps = (x.shape[0] // 8, x.shape[1] // _LANES)
                    return jnp.where(jnp.tile(keep, reps), x, jnp.tile(after, reps))

                piece(gate=gate)


def _kernel(x_hbm, wq_hbm, wk_hbm, wv_hbm, wao_hbm, wup_hbm, dw_hbm, wdn_hbm, wm_hbm,
            o_hbm,
            x_v, wq_v, wk_v, wv_v, wao_v, wupin_v, dw_v, wdn_v, wm_v,
            wvo_v, a_v, wup_v, wo_v, tap_v,
            xa_v, st_v, xq_v, q_v, s_v, p_v, m_v, mx_v, l_v, acc_v,
            u_v, gn_v, cv_v, z_v, ob_v, one_v,
            sems, out_sems,
            *, B, T, D, K):
    M, C, R = _BLK, _CHUNK, _ROWS
    nblk = T // M
    total = B * nblk
    TP = pl.cdiv(T, C) * C
    nchunk = TP // C
    last = nchunk - 1
    nl = D // _LANES
    nc = C // _LANES
    TAIL = T % _LANES
    NR = _norm_rows_per_step(T)
    P = functools.partial
    rows = range(0, M, R)

    def blk_pos(n):
        if isinstance(n, int):
            return n // nblk, (n % nblk) * M
        b = n // nblk
        return b, pl.multiple_of((n - b * nblk) * M, R)

    def xa_rows(r, count):
        return pl.ds(_aligned(r // 2, 8), count // 2)

    def select_rows(n):
        b, r0 = blk_pos(n)
        xq_v[...] = xa_v[xa_rows(b * TP + r0, M), :]

    def q_tile(t):
        q = _dot(_unpack(xq_v[...]), _unpack(a_v[:, _tile(t)]))
        q_v[:, _tile(t)] = _pack(q)
        return q

    def g_tile(t):
        h = _dot(_unpack(xq_v[...]), _unpack(wup_v[:, _tile(nl + t)]))
        gn_v[t] = _gelu(h)
        return h

    def u_tile(t):
        h = _dot(_unpack(xq_v[...]), _unpack(wup_v[:, _tile(t)]))
        u_v[t] = _gelu(h)
        return h

    def qk_tile(n, j, t, mask=False, track_max=False):
        b, _ = blk_pos(n)
        k = _unpack(xa_v[xa_rows(b * TP + j * C + t * _LANES, _LANES), :])
        s = _dot_nt(_unpack(q_v[...]), k)
        if mask:
            col = jax.lax.broadcasted_iota(jnp.int32, s.shape, 1)
            s = jnp.where(col < T - j * C - t * _LANES, s, -jnp.inf)
        s_v[j, :, _tile(t)] = s
        if track_max:
            mx_v[...] = jnp.maximum(mx_v[...], s)
        return s

    def qk_tail(n, i):
        b, _ = blk_pos(n)
        r, count = i * _LANES, min(_LANES, M - i * _LANES)
        q = _unpack(q_v[r // 2:(r + count) // 2, :])
        if count == _LANES:
            s = _dot_nt(_unpack(xa_v[xa_rows(b * TP + T - TAIL, TAIL), :]), q)
            pad = jnp.full((_LANES - TAIL, _LANES), -jnp.inf, _F32)
            s = jnp.concatenate([s, pad], axis=0).T
        else:
            s = _dot_nt(q, _unpack(xa_v[xa_rows(b * TP + T - TAIL, _LANES), :]))
            col = jax.lax.broadcasted_iota(jnp.int32, s.shape, 1)
            s = jnp.where(col < TAIL, s, -jnp.inf)
        s_v[last, r:r + count, _tile(nc - 1)] = s

    def pv_tile(c, j, t, buf, first=False):
        b, _ = blk_pos(c)
        v = _unpack(xa_v[xa_rows(b * TP + j * C, C), _tile(t)])
        pv = _dot(_unpack(p_v[buf * M // 2:(buf + 1) * M // 2, :]), v)
        acc_v[t] = pv if first else acc_v[t] + pv
        return pv

    def out_tile(c, t):
        b, r0 = blk_pos(c)
        out = _dot(_unpack(z_v[...]), _unpack(wo_v[:, _tile(t)]))
        xr = x_v[pl.ds(_aligned(b * T + r0, R), M), _tile(t)].astype(_F32)
        ob_v[c % 2, :, _tile(t)] = (xr + out).astype(ob_v.dtype)
        return out

    def out_copy(c):
        dst = o_hbm.at[pl.ds(_aligned(c * M, R), M)]
        return pltpu.make_async_copy(ob_v.at[c % 2], dst, out_sems.at[c % 2])

    def norm_rows(src_ref, dst_ref, r, gate=_no_gate):
        xs = gate(src_ref[r:r + R, :].astype(_F32))
        dst_ref[r // 2:(r + R) // 2, :] = _pack(_layernorm(xs))

    def g_norm(r, gate=_no_gate):
        g = gate(jnp.concatenate([gn_v[t, r:r + R, :] for t in range(nl)], axis=1))
        g = _layernorm(g)
        for t in range(nl):
            gn_v[t, r:r + R, :] = g[:, _tile(t)]

    def publish_max(r, mx):
        m_v[r:r + R, :] = jnp.broadcast_to(jnp.max(mx, axis=-1, keepdims=True), mx.shape)

    def max_rows(j, r, gate=_no_gate):
        mx = gate(s_v[j, r:r + R, _tile(0)])
        if j > 0:
            mx = jnp.maximum(mx, mx_v[r:r + R, :])
        for t in range(1, nc):
            mx = jnp.maximum(mx, s_v[j, r:r + R, _tile(t)])
        if j == last:
            publish_max(r, mx)
        else:
            mx_v[r:r + R, :] = mx

    def exp_rows(j, buf, r, first=False, gate=_no_gate):
        p = jnp.exp2(s_v[j, r:r + R, :] - jnp.tile(gate(m_v[r:r + R, :]), (1, nc)))
        l = None if first else l_v[r:r + R, :]
        for t in range(nc):
            l = p[:, _tile(t)] if l is None else l + p[:, _tile(t)]
        p_v[(buf * M + r) // 2:(buf * M + r + R) // 2, :] = _pack(p)
        l_v[r:r + R, :] = l

    def scale_rows(r, gate=_no_gate):
        inv = 1.0 / jnp.sum(gate(l_v[r:r + R, :]), axis=-1, keepdims=True)
        for t in range(nl):
            z_v[r // 2:(r + R) // 2, _tile(nl + t)] = _pack(acc_v[t, r:r + R, :] * inv)

    def conv_rows(t, r, gate=_no_gate):
        off = _HALO - K // 2
        conv = None
        for shift in range(8):
            taps = [i for i in range(K) if (off + i) % 8 == shift]
            span = (off + taps[-1]) // 8 * 8
            slab = cv_v[t, pl.ds(r + shift, R + span), :]
            for i in taps:
                a = (off + i) // 8 * 8
                term = slab[a:a + R] * jnp.tile(gate(tap_v[t, i]), (R // 8, 1))
                conv = term if conv is None else conv + term
        return _pack(u_v[t, r:r + R, :] * conv)

    def conv_to_merge(t, r, gate=_no_gate):
        z_v[r // 2:(r + R) // 2, _tile(t)] = conv_rows(t, r, gate)

    def window_head(n, gate=_no_gate):
        _, r0 = blk_pos(n)
        for t in range(nl):
            cv_v[t, _HALO + M:, :] = jnp.where(r0 > 0, gn_v[t, :_HALO, :], 0.0)

    def advance_window(n):
        _, r0 = blk_pos(n)
        for t in range(nl):
            if isinstance(n, int):
                cv_v[t, :_HALO, :] = jnp.zeros((_HALO, _LANES), _F32)
            else:
                cv_v[t, :_HALO, :] = jnp.where(r0 > 0, cv_v[t, M:M + _HALO, :], 0.0)
            cv_v[t, _HALO:_HALO + M, :] = gn_v[t]

    def first_step():
        def fetch(src, dst, i):
            return pltpu.make_async_copy(src, dst, sems.at[i])

        def fetch_x(j):
            part = pl.ds(_aligned(j * C, C), C)
            return fetch(x_hbm.at[part], x_v.at[part], 10 + j)

        halves = [pl.ds(h * D // 2, D // 2) for h in range(2)]
        rest = pl.ds(TP, B * T - TP)
        c_wk = fetch(wk_hbm, wk_v, 0)
        c_wq = [fetch(wq_hbm.at[h], wq_v.at[h], 1 + i) for i, h in enumerate(halves)]
        c_wup = fetch(wup_hbm, wupin_v, 3)
        c_late = [fetch(wv_hbm, wv_v, 4), fetch(wao_hbm, wao_v, 5), fetch(wdn_hbm, wdn_v, 6),
                  fetch(wm_hbm, wm_v, 7), fetch(dw_hbm, dw_v, 8)]
        c_rest = fetch(x_hbm.at[rest], x_v.at[rest], 9)
        for copy in ([c_wk] + c_wq + [fetch_x(0), c_wup] + [fetch_x(j) for j in range(1, nchunk)]
                     + c_late + [c_rest]):
            copy.start()

        one_v[...] = jnp.ones(one_v.shape, jnp.int32)
        mx_v[...] = jnp.full(mx_v.shape, -jnp.inf, _F32)

        def a_tile(h, t):
            a = _dot_nt(wq_v[halves[h]], wk_v[_tile(t), :])
            a = a * (float(D) ** -0.5 * math.log2(math.e))
            a_v[h * D // 4:(h + 1) * D // 4, _tile(t)] = _pack(a)
            return a

        c_wk.wait()
        c_wq[0].wait()
        for t in range(nl):
            a_tile(0, t)
        c_wq[1].wait()
        fetch_x(0).wait()
        plan = _Plan(one_v)
        plan.add("a", [P(a_tile, 1, t) for t in range(nl)])
        plan.spread([P(norm_rows, x_v, xa_v, r) for r in range(0, C, R)], "a", skip=2)
        plan.run()
        select_rows(0)
        for t in range(nl):
            q_tile(t)
        c_wup.wait()
        wup_v[...] = pltpu.bitcast(wupin_v[...], _U32)
        plan = _Plan(one_v)
        plan.add("g", [P(g_tile, t) for t in range(nl)])
        plan.add("u", [P(u_tile, t) for t in range(nl)])
        plan.spread([P(g_norm, r) for r in rows], "u", skip=1)
        plan.run()
        advance_window(0)

        def logits_body(it, carry):
            for jj in range(_UNROLL):
                j = it * _UNROLL + jj
                if jj + 1 < _UNROLL:
                    fetch_x(j + 1).wait()
                else:
                    pl.when(j + 1 < nchunk)(lambda: fetch_x(j + 1).wait())
            plan = _Plan(one_v)
            for jj in range(_UNROLL):
                j = it * _UNROLL + jj
                plan.add(jj, [P(qk_tile, 0, j, t, jj + 1 == _UNROLL and t + 1 == nc, True)
                              for t in range(nc)])
                nxt = jnp.minimum(j + 1, last)
                src = x_v.at[pl.ds(_aligned(nxt * C, R), C)]
                dst = xa_v.at[pl.ds(_aligned(nxt * (C // 2), 8), C // 2)]
                plan.spread([P(norm_rows, src, dst, r) for r in range(0, C, R)], jj, skip=2, defer=True)
            plan.run()
            return carry

        jax.lax.fori_loop(0, nchunk // _UNROLL, logits_body, 0)
        for copy in c_late:
            copy.wait()

        def wvo_tile(t):
            w = _dot(wv_v[...], wao_v[:, _tile(t)])
            wvo_v[:, _tile(t)] = w.astype(_BF16)
            return w

        def wo_tile(lhs_ref, src, dst, t):
            w = _dot(lhs_ref[...], wm_v[src * D:(src + 1) * D, _tile(t)])
            wo_v[dst * D // 2:(dst + 1) * D // 2, _tile(t)] = _pack(w)
            return w

        def spread_taps(t, gate):
            w = dw_v[:, _tile(t)].astype(_F32)
            for i in range(K):
                tap_v[t, i] = jnp.broadcast_to(w[i:i + 1], (8, _LANES))

        plan = _Plan(one_v)
        plan.add("vo", [P(wvo_tile, t) for t in range(nl)])
        plan.add("dm", [P(wo_tile, wdn_v, 1, 0, t) for t in range(nl)])
        plan.add("vom", [P(wo_tile, wvo_v, 0, 1, t) for t in range(nl)])
        plan.spread([lambda gate, r=r: publish_max(r, gate(mx_v[r:r + R, :])) for r in rows], "vo")
        plan.spread([P(spread_taps, t) for t in range(nl)], "dm")
        plan.run()
        for b in range(B):
            xa_v[xa_rows(b * TP + T, TP - T), :] = jnp.zeros(((TP - T) // 2, D), _U32)
        st_v[...] = jnp.zeros(st_v.shape, _U32)
        select_rows(1)
        c_rest.wait()

    def middle_step(n, carry):
        c = n - 1
        pl.when(c >= 2)(lambda: out_copy(c - 2).wait())

        plan = _Plan(one_v)
        plan.add("q", [P(q_tile, t) for t in range(nl)])
        plan.add(("pv", 0), [P(pv_tile, c, 0, t, 0, True) for t in range(nl)])
        plan.add("g", [P(g_tile, t) for t in range(nl)])
        for j in range(last):
            plan.add(("qk", j), [P(qk_tile, n, j, t) for t in range(nc)])
            plan.add(("pv", j + 1), [P(pv_tile, c, j + 1, t, (j + 1) % 2) for t in range(nl)])
        plan.insert([P(qk_tail, n, i) for i in range(pl.cdiv(M, _LANES))], ("pv", last))
        plan.add(("qk", last), [P(qk_tile, n, last, t) for t in range(nc - 1)])
        plan.add("u", [P(u_tile, t) for t in range(nl)])
        plan.add("out", [P(out_tile, c, t) for t in range(nl)])

        for j in range(last):
            plan.spread([P(exp_rows, j + 1, (j + 1) % 2, r) for r in rows], ("pv", j), ("qk", j))
            plan.spread([P(max_rows, j, r) for r in rows], ("pv", j + 1))
        plan.spread([P(g_norm, rows[0]), P(window_head, n)] + [P(g_norm, r) for r in rows[1:]],
                    ("qk", 0), ("pv", 1))
        plan.spread([P(conv_to_merge, t, r) for r in rows for t in range(nl)],
                    *[name for j in range(1, last - 1) for name in (("qk", j), ("pv", j + 1))])
        plan.spread([P(scale_rows, r) for r in rows], ("qk", last))
        plan.spread([P(max_rows, last, r) for r in rows], "out", skip=1)

        def piece(i):
            return jnp.clip(i * (NR // 2), 0, (T - NR) // 2)

        xa_v[pl.ds(_aligned(TP // 2 + piece(c - 1), 8), NR // 2), :] = st_v[...]
        src = x_v.at[pl.ds(_aligned(T + 2 * piece(c), R), NR)]
        plan.spread([P(norm_rows, src, st_v, r) for r in range(0, NR, R)], ("pv", 0), "g")

        for r in rows:
            exp_rows(0, 0, r, True)
        plan.run()
        select_rows(jnp.minimum(n + 1, total - 1))
        advance_window(n)
        out_copy(c).start()
        return carry

    def last_step():
        c = total - 1
        iters = nchunk // _UNROLL
        out_copy(c - 2).wait()
        for t in range(nl):
            cv_v[t, _HALO + M:, :] = jnp.zeros((_HALO, _LANES), _F32)
        l_v[...] = jnp.zeros(l_v.shape, _F32)
        acc_v[...] = jnp.zeros(acc_v.shape, _F32)

        def conv_to_stash(t, r, gate):
            gn_v[t, r // 2:(r + R) // 2, :] = pltpu.bitcast(conv_rows(t, r, gate), _F32)

        def values_body(it, carry):
            plan = _Plan(one_v)
            for jj in range(_UNROLL):
                j = it * _UNROLL + jj
                plan.add(jj, [P(pv_tile, c, j, t, jj % 2) for t in range(nl)])
                if jj + 1 < _UNROLL:
                    plan.spread([P(exp_rows, j + 1, (jj + 1) % 2, r) for r in rows], jj, skip=1)
            plan.spread([P(conv_to_stash, it * (nl // iters) + t, r)
                         for t in range(nl // iters) for r in rows], *range(_UNROLL), skip=1)
            for r in rows:
                exp_rows(it * _UNROLL, 0, r)
            plan.run()
            return carry

        jax.lax.fori_loop(0, iters, values_body, 0)
        for t in range(nl):
            z_v[:, _tile(t)] = pltpu.bitcast(gn_v[t, :M // 2, :], _U32)
        for r in rows:
            scale_rows(r)
        final = [pltpu.make_async_copy(ob_v.at[c % 2, :, _tile(t)],
                                       o_hbm.at[pl.ds(c * M, M), _tile(t)], sems.at[t])
                 for t in range(nl)]
        for t in range(nl):
            out_tile(c, t)
            final[t].start()
        out_copy(c - 1).wait()
        for copy in final:
            copy.wait()

    first_step()
    jax.lax.fori_loop(1, total, middle_step, 0)
    last_step()


@jax.jit
def pallas_standalone__conformer_family_branchformer__speech_kernel(
    x: jax.Array,
    w_q: jax.Array,
    w_k: jax.Array,
    w_v: jax.Array,
    w_ao: jax.Array,
    w_up: jax.Array,
    dw: jax.Array,
    w_dn: jax.Array,
    w_merge: jax.Array,
):
    B, T, D = x.shape
    K = dw.shape[0]
    M, C = _BLK, _CHUNK
    TP = pl.cdiv(T, C) * C
    nl = D // _LANES
    assert B == 2 and T % M == 0 and D % _LANES == 0 and K // 2 < _HALO
    assert TP - T + T % _LANES == _LANES and (T % _LANES) % _ROWS == 0
    weights = (w_q, w_k, w_v, w_ao, w_up, dw, w_dn, w_merge)
    assert all(a.dtype == _BF16 for a in (x,) + weights)

    vmem = pltpu.VMEM
    out = pl.pallas_call(
        functools.partial(_kernel, B=B, T=T, D=D, K=K),
        in_specs=[pl.BlockSpec(memory_space=pl.ANY)] * 9,
        out_specs=pl.BlockSpec(memory_space=pl.ANY),
        out_shape=jax.ShapeDtypeStruct((B * T, D), x.dtype),
        scratch_shapes=[
            vmem((B * T, D), x.dtype),
            *[vmem(w.shape, w.dtype) for w in weights],
            vmem((D, D), _BF16),
            vmem((D // 2, D), _U32),
            vmem((D // 2, 2 * D), _U32),
            vmem((D, D), _U32),
            vmem((nl, K, 8, _LANES), _F32),
            vmem((B * TP // 2, D), _U32),
            vmem((_norm_rows_per_step(T) // 2, D), _U32),
            vmem((M // 2, D), _U32),
            vmem((M // 2, D), _U32),
            vmem((TP // C, M, C), _F32),
            vmem((M, C), _U32),
            vmem((M, _LANES), _F32),
            vmem((M, _LANES), _F32),
            vmem((M, _LANES), _F32),
            vmem((nl, M, _LANES), _F32),
            vmem((nl, M, _LANES), _F32),
            vmem((nl, M, _LANES), _F32),
            vmem((nl, M + 2 * _HALO, _LANES), _F32),
            vmem((M // 2, 2 * D), _U32),
            vmem((2, M, D), x.dtype),
            vmem((8, _LANES), jnp.int32),
            pltpu.SemaphoreType.DMA((10 + TP // C,)),
            pltpu.SemaphoreType.DMA((2,)),
        ],
        compiler_params=pltpu.CompilerParams(vmem_limit_bytes=96 * 2**20),
    )(x.reshape(B * T, D), *weights)
    return out.reshape(B, T, D)
```

```python
import functools
import math

import jax
import jax.numpy as jnp
import jax.experimental.pallas as pl
import jax.experimental.pallas.tpu as pltpu

_EPS = 1e-5
_LANES = 128
_ROWS = 16
_BLK = 400
_CHUNK = 512
_UNROLL = 4
_HALO = 16
_GELU_C = math.sqrt(2.0 / math.pi)

_F32 = jnp.float32
_BF16 = jnp.bfloat16
_U32 = jnp.uint32


def _dot(a, b):
    return jax.lax.dot_general(a, b, (((1,), (0,)), ((), ())), preferred_element_type=_F32)


def _dot_nt(a, b):
    return jax.lax.dot_general(a, b, (((1,), (1,)), ((), ())), preferred_element_type=_F32)


def _pack(x):
    return pltpu.bitcast(x.astype(_BF16), _U32)


def _unpack(w):
    return pltpu.bitcast(w, _BF16)


def _layernorm(x):
    m = jnp.mean(x, axis=-1, keepdims=True)
    xc = x - m
    v = jnp.mean(xc * xc, axis=-1, keepdims=True)
    return xc * jax.lax.rsqrt(v + _EPS)


def _gelu(x):
    inner = x * (_GELU_C + (_GELU_C * 0.044715) * (x * x))
    hx = 0.5 * x
    return hx + hx * jnp.tanh(inner)


def _tile(t):
    return slice(t * _LANES, (t + 1) * _LANES)


def _no_gate(x):
    return x


def _accumulate(first, load, x):
    if isinstance(first, bool):
        return x if first else load() + x
    return jnp.where(first, 0.0, load()) + x


def _aligned(v, mult):
    return v if isinstance(v, int) else pl.multiple_of(v, mult)


def _norm_rows_per_step(T):
    return pl.cdiv(T, _ROWS * (T // _BLK - 1)) * _ROWS


class _Plan:
    def __init__(self, ones_ref):
        self.ones_ref = ones_ref
        self.order = []
        self.slots = {}

    def add(self, name, tasks):
        self.slots[name] = list(range(len(self.order), len(self.order) + len(tasks)))
        self.order += [(task, []) for task in tasks]

    def insert(self, tasks, name):
        for task, slot in zip(tasks, self.slots[name], strict=True):
            self.order[slot][1].append((slot, -1.0, lambda gate, task=task: task()))

    def spread(self, pieces, *names, skip=0, defer=False):
        slots = [i for name in names for i in self.slots[name]]
        for k, piece in enumerate(pieces):
            pos = k * (len(slots) - skip) / len(pieces)
            slot = slots[int(pos)]
            self.order[slots[-1] if defer else slot][1].append((slot, pos - int(pos), piece))

    def run(self):
        keep = self.ones_ref[...] != 0
        results = []
        for task, pieces in self.order:
            results.append(task())
            for slot, frac, piece in sorted(pieces, key=lambda e: e[:2]):
                r = int(max(frac, 0.0) * (results[slot].shape[0] // 8)) * 8

                def gate(x, after=results[slot][r:r + 8]):
                    reps = (x.shape[0] // 8, x.shape[1] // _LANES)
                    return jnp.where(jnp.tile(keep, reps), x, jnp.tile(after, reps))

                piece(gate=gate)


def _kernel(x_hbm, wq_hbm, wk_hbm, wv_hbm, wao_hbm, wup_hbm, dw_hbm, wdn_hbm, wm_hbm,
            o_hbm,
            x_v, wq_v, wk_v, wv_v, wao_v, wupin_v, dw_v, wdn_v, wm_v,
            wvo_v, a_v, wup_v, wo_v, tap_v,
            xa_v, st_v, xq_v, q_v, s_v, p_v, m_v, mx_v, l_v, acc_v,
            u_v, gn_v, cv_v, z_v, ob_v, one_v,
            sems, out_sems,
            *, B, T, D, K):
    M, C, R = _BLK, _CHUNK, _ROWS
    nblk = T // M
    total = B * nblk
    TP = pl.cdiv(T, C) * C
    nchunk = TP // C
    last = nchunk - 1
    nl = D // _LANES
    nc = C // _LANES
    TAIL = T % _LANES
    NR = _norm_rows_per_step(T)
    P = functools.partial
    rows = range(0, M, R)

    def blk_pos(n):
        if isinstance(n, int):
            return n // nblk, (n % nblk) * M
        b = n // nblk
        return b, pl.multiple_of((n - b * nblk) * M, R)

    def xa_rows(r, count):
        return pl.ds(_aligned(r // 2, 8), count // 2)

    def select_rows(n):
        b, r0 = blk_pos(n)
        xq_v[...] = xa_v[xa_rows(b * TP + r0, M), :]

    def q_tile(t):
        q = _dot(_unpack(xq_v[...]), _unpack(a_v[:, _tile(t)]))
        q_v[:, _tile(t)] = _pack(q)
        return q

    def g_tile(t):
        h = _dot(_unpack(xq_v[...]), _unpack(wup_v[:, _tile(nl + t)]))
        gn_v[t] = _gelu(h)
        return h

    def u_tile(t):
        h = _dot(_unpack(xq_v[...]), _unpack(wup_v[:, _tile(t)]))
        u_v[t] = _gelu(h)
        return h

    def qk_tile(n, j, t, mask=False, track_max=False):
        b, _ = blk_pos(n)
        k = _unpack(xa_v[xa_rows(b * TP + j * C + t * _LANES, _LANES), :])
        s = _dot_nt(_unpack(q_v[...]), k)
        if mask:
            col = jax.lax.broadcasted_iota(jnp.int32, s.shape, 1)
            s = jnp.where(col < T - j * C - t * _LANES, s, -jnp.inf)
        s_v[j, :, _tile(t)] = s
        if track_max:
            mx_v[...] = jnp.maximum(mx_v[...], s)
        return s

    def qk_tail(n, i):
        b, _ = blk_pos(n)
        r, count = i * _LANES, min(_LANES, M - i * _LANES)
        q = _unpack(q_v[r // 2:(r + count) // 2, :])
        if count == _LANES:
            s = _dot_nt(_unpack(xa_v[xa_rows(b * TP + T - TAIL, TAIL), :]), q)
            pad = jnp.full((_LANES - TAIL, _LANES), -jnp.inf, _F32)
            s = jnp.concatenate([s, pad], axis=0).T
        else:
            s = _dot_nt(q, _unpack(xa_v[xa_rows(b * TP + T - TAIL, _LANES), :]))
            col = jax.lax.broadcasted_iota(jnp.int32, s.shape, 1)
            s = jnp.where(col < TAIL, s, -jnp.inf)
        s_v[last, r:r + count, _tile(nc - 1)] = s

    def pv_tile(c, j, t, buf, first=False):
        b, _ = blk_pos(c)
        v = _unpack(xa_v[xa_rows(b * TP + j * C, C), _tile(t)])
        pv = _dot(_unpack(p_v[buf * M // 2:(buf + 1) * M // 2, :]), v)
        acc_v[t] = _accumulate(first, lambda: acc_v[t], pv)
        return pv

    def out_tile(c, t):
        b, r0 = blk_pos(c)
        out = _dot(_unpack(z_v[...]), _unpack(wo_v[:, _tile(t)]))
        xr = x_v[pl.ds(_aligned(b * T + r0, R), M), _tile(t)].astype(_F32)
        ob_v[c % 2, :, _tile(t)] = (xr + out).astype(ob_v.dtype)
        return out

    def out_copy(c):
        dst = o_hbm.at[pl.ds(_aligned(c * M, R), M)]
        return pltpu.make_async_copy(ob_v.at[c % 2], dst, out_sems.at[c % 2])

    def norm_rows(src_ref, dst_ref, r, gate=_no_gate):
        xs = gate(src_ref[r:r + R, :].astype(_F32))
        dst_ref[r // 2:(r + R) // 2, :] = _pack(_layernorm(xs))

    def g_norm(r, gate=_no_gate):
        g = gate(jnp.concatenate([gn_v[t, r:r + R, :] for t in range(nl)], axis=1))
        g = _layernorm(g)
        for t in range(nl):
            gn_v[t, r:r + R, :] = g[:, _tile(t)]

    def publish_max(r, mx):
        m_v[r:r + R, :] = jnp.broadcast_to(jnp.max(mx, axis=-1, keepdims=True), mx.shape)

    def max_rows(j, r, gate=_no_gate):
        mx = gate(s_v[j, r:r + R, _tile(0)])
        if j > 0:
            mx = jnp.maximum(mx, mx_v[r:r + R, :])
        for t in range(1, nc):
            mx = jnp.maximum(mx, s_v[j, r:r + R, _tile(t)])
        if j == last:
            publish_max(r, mx)
        else:
            mx_v[r:r + R, :] = mx

    def exp_rows(j, buf, r, first=False, gate=_no_gate):
        p = jnp.exp2(s_v[j, r:r + R, :] - jnp.tile(gate(m_v[r:r + R, :]), (1, nc)))
        l = _accumulate(first, lambda: l_v[r:r + R, :], p[:, _tile(0)])
        for t in range(1, nc):
            l = l + p[:, _tile(t)]
        p_v[(buf * M + r) // 2:(buf * M + r + R) // 2, :] = _pack(p)
        l_v[r:r + R, :] = l

    def scale_rows(r, gate=_no_gate):
        inv = 1.0 / jnp.sum(gate(l_v[r:r + R, :]), axis=-1, keepdims=True)
        for t in range(nl):
            z_v[r // 2:(r + R) // 2, _tile(nl + t)] = _pack(acc_v[t, r:r + R, :] * inv)

    def conv_rows(t, r, gate=_no_gate):
        off = _HALO - K // 2
        conv = None
        for shift in range(8):
            taps = [i for i in range(K) if (off + i) % 8 == shift]
            span = (off + taps[-1]) // 8 * 8
            slab = cv_v[t, pl.ds(r + shift, R + span), :]
            for i in taps:
                a = (off + i) // 8 * 8
                term = slab[a:a + R] * jnp.tile(gate(tap_v[t, i]), (R // 8, 1))
                conv = term if conv is None else conv + term
        return _pack(u_v[t, r:r + R, :] * conv)

    def conv_to_merge(t, r, gate=_no_gate):
        z_v[r // 2:(r + R) // 2, _tile(t)] = conv_rows(t, r, gate)

    def window_head(n, gate=_no_gate):
        _, r0 = blk_pos(n)
        for t in range(nl):
            cv_v[t, _HALO + M:, :] = jnp.where(r0 > 0, gn_v[t, :_HALO, :], 0.0)

    def advance_window(n):
        _, r0 = blk_pos(n)
        for t in range(nl):
            if isinstance(n, int):
                cv_v[t, :_HALO, :] = jnp.zeros((_HALO, _LANES), _F32)
            else:
                cv_v[t, :_HALO, :] = jnp.where(r0 > 0, cv_v[t, M:M + _HALO, :], 0.0)
            cv_v[t, _HALO:_HALO + M, :] = gn_v[t]

    def first_step():
        def fetch(src, dst, i):
            return pltpu.make_async_copy(src, dst, sems.at[i])

        def fetch_x(j):
            part = pl.ds(_aligned(j * C, C), C)
            return fetch(x_hbm.at[part], x_v.at[part], 10 + j)

        halves = [pl.ds(h * D // 2, D // 2) for h in range(2)]
        rest = pl.ds(TP, B * T - TP)
        c_wk = fetch(wk_hbm, wk_v, 0)
        c_wq = [fetch(wq_hbm.at[h], wq_v.at[h], 1 + i) for i, h in enumerate(halves)]
        c_wup = fetch(wup_hbm, wupin_v, 3)
        c_late = [fetch(wv_hbm, wv_v, 4), fetch(wao_hbm, wao_v, 5), fetch(wdn_hbm, wdn_v, 6),
                  fetch(wm_hbm, wm_v, 7), fetch(dw_hbm, dw_v, 8)]
        c_rest = fetch(x_hbm.at[rest], x_v.at[rest], 9)
        for copy in ([c_wk] + c_wq + [fetch_x(0), c_wup] + [fetch_x(j) for j in range(1, nchunk)]
                     + c_late + [c_rest]):
            copy.start()

        one_v[...] = jnp.ones(one_v.shape, jnp.int32)
        mx_v[...] = jnp.full(mx_v.shape, -jnp.inf, _F32)

        def a_tile(h, t):
            a = _dot_nt(wq_v[halves[h]], wk_v[_tile(t), :])
            a = a * (float(D) ** -0.5 * math.log2(math.e))
            a_v[h * D // 4:(h + 1) * D // 4, _tile(t)] = _pack(a)
            return a

        c_wk.wait()
        c_wq[0].wait()
        for t in range(nl):
            a_tile(0, t)
        c_wq[1].wait()
        fetch_x(0).wait()
        plan = _Plan(one_v)
        plan.add("a", [P(a_tile, 1, t) for t in range(nl)])
        plan.spread([P(norm_rows, x_v, xa_v, r) for r in range(0, C, R)], "a", skip=2)
        plan.run()
        select_rows(0)
        for t in range(nl):
            q_tile(t)
        c_wup.wait()
        wup_v[...] = pltpu.bitcast(wupin_v[...], _U32)
        plan = _Plan(one_v)
        plan.add("g", [P(g_tile, t) for t in range(nl)])
        plan.add("u", [P(u_tile, t) for t in range(nl)])
        plan.spread([P(g_norm, r) for r in rows], "u", skip=1)
        plan.run()
        advance_window(0)

        def logits_body(it, carry):
            for jj in range(_UNROLL):
                j = it * _UNROLL + jj
                if jj + 1 < _UNROLL:
                    fetch_x(j + 1).wait()
                else:
                    pl.when(j + 1 < nchunk)(lambda: fetch_x(j + 1).wait())
            plan = _Plan(one_v)
            for jj in range(_UNROLL):
                j = it * _UNROLL + jj
                plan.add(jj, [P(qk_tile, 0, j, t, jj + 1 == _UNROLL and t + 1 == nc, True)
                              for t in range(nc)])
                nxt = jnp.minimum(j + 1, last)
                src = x_v.at[pl.ds(_aligned(nxt * C, R), C)]
                dst = xa_v.at[pl.ds(_aligned(nxt * (C // 2), 8), C // 2)]
                plan.spread([P(norm_rows, src, dst, r) for r in range(0, C, R)], jj, skip=2, defer=True)
            plan.run()
            return carry

        jax.lax.fori_loop(0, nchunk // _UNROLL, logits_body, 0)
        for copy in c_late:
            copy.wait()

        def wvo_tile(t):
            w = _dot(wv_v[...], wao_v[:, _tile(t)])
            wvo_v[:, _tile(t)] = w.astype(_BF16)
            return w

        def wo_tile(lhs_ref, src, dst, t):
            w = _dot(lhs_ref[...], wm_v[src * D:(src + 1) * D, _tile(t)])
            wo_v[dst * D // 2:(dst + 1) * D // 2, _tile(t)] = _pack(w)
            return w

        def spread_taps(t, gate):
            w = dw_v[:, _tile(t)].astype(_F32)
            for i in range(K):
                tap_v[t, i] = jnp.broadcast_to(w[i:i + 1], (8, _LANES))

        def clear_staged(r, gate):
            st_v[r:r + 8, :] = pltpu.bitcast(gate(jnp.zeros((8, D), _F32)), _U32)

        plan = _Plan(one_v)
        plan.add("vo", [P(wvo_tile, t) for t in range(nl)])
        plan.add("dm", [P(wo_tile, wdn_v, 1, 0, t) for t in range(nl)])
        plan.add("vom", [P(wo_tile, wvo_v, 0, 1, t) for t in range(nl)])
        plan.spread([lambda gate, r=r: publish_max(r, gate(mx_v[r:r + R, :])) for r in rows], "vo")
        plan.spread([P(spread_taps, t) for t in range(nl)], "dm")
        plan.spread([P(clear_staged, r) for r in range(0, NR // 2, 8)], "vom")
        plan.run()
        for b in range(B):
            xa_v[xa_rows(b * TP + T, TP - T), :] = jnp.zeros(((TP - T) // 2, D), _U32)
        select_rows(1)
        c_rest.wait()

    def middle_step(n, carry):
        c = n - 1
        pl.when(c >= 2)(lambda: out_copy(c - 2).wait())

        plan = _Plan(one_v)
        plan.add("q", [P(q_tile, t) for t in range(nl)])
        plan.add(("pv", 0), [P(pv_tile, c, 0, t, 0, True) for t in range(nl)])
        plan.add("g", [P(g_tile, t) for t in range(nl)])
        for j in range(last):
            plan.add(("qk", j), [P(qk_tile, n, j, t) for t in range(nc)])
            plan.add(("pv", j + 1), [P(pv_tile, c, j + 1, t, (j + 1) % 2) for t in range(nl)])
        plan.insert([P(qk_tail, n, i) for i in range(pl.cdiv(M, _LANES))], ("pv", last))
        plan.add(("qk", last), [P(qk_tile, n, last, t) for t in range(nc - 1)])
        plan.add("u", [P(u_tile, t) for t in range(nl)])
        plan.add("out", [P(out_tile, c, t) for t in range(nl)])

        for j in range(last):
            plan.spread([P(exp_rows, j + 1, (j + 1) % 2, r) for r in rows], ("pv", j), ("qk", j))
            plan.spread([P(max_rows, j, r) for r in rows], ("pv", j + 1))
        plan.spread([P(g_norm, rows[0]), P(window_head, n)] + [P(g_norm, r) for r in rows[1:]],
                    ("qk", 0), ("pv", 1))
        plan.spread([P(conv_to_merge, t, r) for r in rows for t in range(nl)],
                    *[name for j in range(1, last - 1) for name in (("qk", j), ("pv", j + 1))])
        plan.spread([P(scale_rows, r) for r in rows], ("qk", last))
        plan.spread([P(max_rows, last, r) for r in rows], "out", skip=1)

        def piece(i):
            return jnp.clip(i * (NR // 2), 0, (T - NR) // 2)

        xa_v[pl.ds(_aligned(TP // 2 + piece(c - 1), 8), NR // 2), :] = st_v[...]
        src = x_v.at[pl.ds(_aligned(T + 2 * piece(c), R), NR)]
        plan.spread([P(norm_rows, src, st_v, r) for r in range(0, NR, R)], "q", ("pv", 0))

        for r in rows:
            exp_rows(0, 0, r, True)
        plan.run()
        select_rows(jnp.minimum(n + 1, total - 1))
        advance_window(n)
        out_copy(c).start()
        return carry

    def last_step():
        c = total - 1
        iters = nchunk // _UNROLL
        out_copy(c - 2).wait()
        for t in range(nl):
            cv_v[t, _HALO + M:, :] = jnp.zeros((_HALO, _LANES), _F32)

        def conv_to_stash(t, r, gate):
            gn_v[t, r // 2:(r + R) // 2, :] = pltpu.bitcast(conv_rows(t, r, gate), _F32)

        def values_body(it, carry):
            plan = _Plan(one_v)
            for jj in range(_UNROLL):
                j = it * _UNROLL + jj
                plan.add(jj, [P(pv_tile, c, j, t, jj % 2, it == 0 if jj == 0 else False) for t in range(nl)])
                if jj + 1 < _UNROLL:
                    plan.spread([P(exp_rows, j + 1, (jj + 1) % 2, r) for r in rows], jj, skip=1)
            plan.spread([P(conv_to_stash, it * (nl // iters) + t, r)
                         for t in range(nl // iters) for r in rows], *range(_UNROLL), skip=1)
            for r in rows:
                exp_rows(it * _UNROLL, 0, r, it == 0)
            plan.run()
            return carry

        jax.lax.fori_loop(0, iters, values_body, 0)
        for t in range(nl):
            z_v[:, _tile(t)] = pltpu.bitcast(gn_v[t, :M // 2, :], _U32)
        for r in rows:
            scale_rows(r)
        final = [pltpu.make_async_copy(ob_v.at[c % 2, :, _tile(t)],
                                       o_hbm.at[pl.ds(c * M, M), _tile(t)], sems.at[t])
                 for t in range(nl)]
        for t in range(nl):
            out_tile(c, t)
            final[t].start()
        out_copy(c - 1).wait()
        for copy in final:
            copy.wait()

    first_step()
    jax.lax.fori_loop(1, total, middle_step, 0)
    last_step()


@jax.jit
def pallas_standalone__conformer_family_branchformer__speech_kernel(
    x: jax.Array,
    w_q: jax.Array,
    w_k: jax.Array,
    w_v: jax.Array,
    w_ao: jax.Array,
    w_up: jax.Array,
    dw: jax.Array,
    w_dn: jax.Array,
    w_merge: jax.Array,
):
    B, T, D = x.shape
    K = dw.shape[0]
    M, C = _BLK, _CHUNK
    TP = pl.cdiv(T, C) * C
    nl = D // _LANES
    assert B == 2 and T % M == 0 and D % _LANES == 0 and K // 2 < _HALO
    assert TP - T + T % _LANES == _LANES and (T % _LANES) % _ROWS == 0
    weights = (w_q, w_k, w_v, w_ao, w_up, dw, w_dn, w_merge)
    assert all(a.dtype == _BF16 for a in (x,) + weights)

    vmem = pltpu.VMEM
    out = pl.pallas_call(
        functools.partial(_kernel, B=B, T=T, D=D, K=K),
        in_specs=[pl.BlockSpec(memory_space=pl.ANY)] * 9,
        out_specs=pl.BlockSpec(memory_space=pl.ANY),
        out_shape=jax.ShapeDtypeStruct((B * T, D), x.dtype),
        scratch_shapes=[
            vmem((B * T, D), x.dtype),
            *[vmem(w.shape, w.dtype) for w in weights],
            vmem((D, D), _BF16),
            vmem((D // 2, D), _U32),
            vmem((D // 2, 2 * D), _U32),
            vmem((D, D), _U32),
            vmem((nl, K, 8, _LANES), _F32),
            vmem((B * TP // 2, D), _U32),
            vmem((_norm_rows_per_step(T) // 2, D), _U32),
            vmem((M // 2, D), _U32),
            vmem((M // 2, D), _U32),
            vmem((TP // C, M, C), _F32),
            vmem((M, C), _U32),
            vmem((M, _LANES), _F32),
            vmem((M, _LANES), _F32),
            vmem((M, _LANES), _F32),
            vmem((nl, M, _LANES), _F32),
            vmem((nl, M, _LANES), _F32),
            vmem((nl, M, _LANES), _F32),
            vmem((nl, M + 2 * _HALO, _LANES), _F32),
            vmem((M // 2, 2 * D), _U32),
            vmem((2, M, D), x.dtype),
            vmem((8, _LANES), jnp.int32),
            pltpu.SemaphoreType.DMA((10 + TP // C,)),
            pltpu.SemaphoreType.DMA((2,)),
        ],
        compiler_params=pltpu.CompilerParams(vmem_limit_bytes=96 * 2**20),
    )(x.reshape(B * T, D), *weights)
    return out.reshape(B, T, D)
```
